```python
import os as _os
_os.environ.setdefault("JAX_PLATFORMS", "cpu")
import jax
import jax.numpy as jnp

def _softmax(x, axis=-1):
    return jax.nn.softmax(x, axis=axis)
def _gelu(x):
    return jax.nn.gelu(x, approximate=True)
def _silu(x):
    return jax.nn.silu(x)
def _sigmoid(x):
    return jax.nn.sigmoid(x)
def _layernorm(x, axis=-1, eps=1e-5):
    m = jnp.mean(x, axis=axis, keepdims=True)
    v = jnp.var(x, axis=axis, keepdims=True)
    return (x - m) / jnp.sqrt(v + eps)
def _scatter_add(tgt, idx, src, axis=0):
    return tgt.at[idx].add(src)
def _segment_sum(src, seg, n):
    return jax.ops.segment_sum(src, seg, n)
class _Rng:
    def __init__(self, key):
        self._k = key
    def _next(self):
        self._k, sub = jax.random.split(self._k)
        return sub
    def normal(self, shape):
        return jax.random.normal(self._next(), shape, dtype=jnp.bfloat16)
    def randint(self, lo, hi, shape):
        return jax.random.randint(self._next(), shape, lo, hi, dtype=jnp.int32)
    def uniform(self, shape, lo=0.0, hi=1.0):
        return jax.random.uniform(self._next(), shape, jnp.bfloat16, lo, hi)
    def permutation(self, n):
        return jax.random.permutation(self._next(), n)


kernel_name = 'gated_mix__softmax_full_mha__dense_activation_relu__prompt'

def setup_inputs():
    _rng = _Rng(jax.random.key(int.from_bytes(__import__("os").urandom(4), "little")))
    _w = (lambda a: (lambda t: t.astype(jnp.bfloat16) if jnp.issubdtype(t.dtype, jnp.floating) else t)(jnp.asarray(a)))
    def _A_setup():
        B, S, D = 1, 2048, 640
        return {
            "x": _w((lambda *s: _rng.normal(s) * 0.05)(B, S, D)),
            "wqkv": _w((lambda *s: _rng.normal(s) * 0.8)(D, 3 * D)),
            "wo": _w((lambda *s: _rng.normal(s) * 0.05)(D, D)),
        }
    _A_in = _A_setup()

    def _B_setup():
        B, S, D, Dff = 1, 2048, 640, 1536
        return {
            "x": _w((lambda *s: _rng.normal(s) * 0.05)(B, S, D)),
            "w1": _w((lambda *s: _rng.normal(s) * 0.05)(D, Dff)),
            "w2": _w((lambda *s: _rng.normal(s) * 0.05)(Dff, D)),
        }
    _B_in = _B_setup()

    return {
        "A_x": _A_in["x"],
        "A_wqkv": _A_in["wqkv"],
        "A_wo": _A_in["wo"],
        "B_x": _B_in["x"],
        "B_w1": _B_in["w1"],
        "B_w2": _B_in["w2"],
        "gate_w": _w((lambda *s: _rng.normal(s) * 0.05)(640) * 16.0),
    }

def reference(A_x, A_wqkv, A_wo, B_x, B_w1, B_w2, gate_w):
    def _A_ref(x, wqkv, wo):
        B, S, D = x.shape
        H = 32; Dh = D // H
        qkv = (lambda x, *d: x.transpose(*d))((x @ wqkv).reshape(B, S, 3, H, Dh), 2, 0, 3, 1, 4)
        q, k, v = qkv[0], qkv[1], qkv[2]
        scale = Dh ** -0.5
        scores = jnp.einsum("bhqd,bhkd->bhqk", q, k) * scale
        p = _softmax(scores, axis=-1)
        o = jnp.einsum("bhqk,bhkd->bhqd", p, v)
        return (lambda x, *d: x.transpose(*d))(o, 0, 2, 1, 3).reshape(B, S, D) @ wo

    def _B_ref(x, w1, w2):
        h = jnp.einsum("bsd,df->bsf", x, w1)
        zero = jnp.zeros_like(h)
        h = jnp.maximum(h, zero)
        return jnp.einsum("bsf,fd->bsd", h, w2)

    x = A_x
    g = _sigmoid((x * gate_w).sum(-1, keepdims=True))
    a = _A_ref(x, A_wqkv, A_wo)
    b = _B_ref(x, B_w1, B_w2)
    return g * a + (1 - g) * b
```

```python
import functools
import math
import jax
import jax.numpy as jnp
from jax import lax
import jax.experimental.pallas as pl
import jax.experimental.pallas.tpu as pltpu

S = 2048
D = 640
H = 32
DH = 20
DFF = 1536
NWIN = 6
VROWS = 24

NT = (((1,), (1,)), ((), ()))
NN = (((1,), (0,)), ((), ()))
TN = (((0,), (1,)), ((), ()))


def _window(a, w):
    c0 = 120 * w
    g0 = c0 // 128
    g1 = min(c0 + 119, D - 1) // 128
    lo = a[:, g0 * 128:(g0 + 1) * 128]
    if g1 == g0:
        return lo
    hi = a[:, g1 * 128:(g1 + 1) * 128]
    lane = lax.broadcasted_iota(jnp.int32, lo.shape, 1)
    return jnp.where(lane >= (c0 % 128), lo, hi)


def make_kernel(BQ=512, RC=512, BO=512, KC=128):
    NQ = S // BQ
    NITEM = NQ * H
    NO = S // BO
    qscale = (DH ** -0.5) * math.log2(math.e)

    def kernel(x_ref, wqkv_ref, wo_ref, w1_ref, w2_ref, gw_ref, o_ref,
               kwin_ref, vt_ref, qwin_ref, ot_ref, sa_ref, sb_ref, ma_ref, mb_ref):
        i = pl.program_id(0)

        @pl.when(i == 0)
        def _():
            def proj(c, carry):
                r0 = pl.multiple_of(c * RC, RC)
                xc = x_ref[pl.ds(r0, RC), :]
                q = jnp.dot(xc, wqkv_ref[:, 0:D], preferred_element_type=jnp.float32) * qscale
                for w in range(NWIN):
                    qwin_ref[w, pl.ds(r0, RC), :] = _window(q, w)
                k = jnp.dot(xc, wqkv_ref[:, D:2 * D], preferred_element_type=jnp.float32)
                for w in range(NWIN):
                    kwin_ref[w, pl.ds(r0, RC), :] = _window(k, w).astype(jnp.bfloat16)
                vt = lax.dot_general(wqkv_ref[:, 2 * D:3 * D], xc, TN, preferred_element_type=jnp.float32)
                row = lax.broadcasted_iota(jnp.int32, (VROWS, RC), 0)
                for h in range(H):
                    st = (DH * h) // 8 * 8
                    off = DH * h - st
                    blk = vt[st:st + VROWS, :]
                    blk = jnp.where((row >= off) & (row < off + DH), blk, 1.0)
                    vt_ref[h, :, pl.ds(r0, RC)] = blk
                return carry
            lax.fori_loop(0, S // RC, proj, 0)

            lane = lax.broadcasted_iota(jnp.int32, (BQ, 128), 1)

            def masked_q(t):
                h = t % H
                qb = t // H
                w = h // 6
                off = (DH * h) % 128
                rel = (lane - off) & 127
                q0 = pl.multiple_of(qb * BQ, BQ)
                return w, jnp.where(rel < DH, qwin_ref[w, pl.ds(q0, BQ), :], 0.0).astype(jnp.bfloat16)

            def stage(t_next, s_next, m_next, t_cur, s_cur, m_cur):
                if t_next is not None:
                    w, qm = masked_q(t_next)
                    mx = None
                if t_cur is not None:
                    h = t_cur % H
                    q0 = pl.multiple_of((t_cur // H) * BQ, BQ)
                    m = m_cur[0:1, :]
                    acc = None
                for c in range(S // KC):
                    ks = slice(c * KC, (c + 1) * KC)
                    if t_next is not None:
                        s = lax.dot_general(kwin_ref[w, ks, :], qm, NT, preferred_element_type=jnp.float32)
                        s_next[ks, :] = s
                        cm = jnp.max(s.reshape(KC // 8, 8, BQ), axis=0)
                        mx = cm if mx is None else jnp.maximum(mx, cm)
                    if t_cur is not None:
                        p = jnp.exp2(s_cur[ks, :] - m)
                        pv = lax.dot_general(vt_ref[h, :, ks], p, NN, preferred_element_type=jnp.float32)
                        acc = pv if acc is None else acc + pv
                if t_next is not None:
                    m_next[...] = jnp.broadcast_to(jnp.max(mx, axis=0, keepdims=True), (8, BQ))
                if t_cur is not None:
                    ot_ref[h, :, pl.ds(q0, BQ)] = acc

            stage(0, sa_ref, ma_ref, None, None, None)

            def body(u, carry):
                t = 2 * u
                stage(t + 1, sb_ref, mb_ref, t, sa_ref, ma_ref)
                stage(t + 2, sa_ref, ma_ref, t + 1, sb_ref, mb_ref)
                return carry
            lax.fori_loop(0, NITEM // 2 - 1, body, 0)
            stage(NITEM - 1, sb_ref, mb_ref, NITEM - 2, sa_ref, ma_ref)
            stage(None, None, None, NITEM - 1, sb_ref, mb_ref)

        r0 = pl.multiple_of(i * BO, BO)
        xq = x_ref[pl.ds(r0, BO), :]
        row8 = lax.broadcasted_iota(jnp.int32, (8, BO), 0)
        pieces = []
        for pair in range(H // 2):
            he, ho = 2 * pair, 2 * pair + 1
            ae = ot_ref[he, :, pl.ds(r0, BO)]
            ao = ot_ref[ho, :, pl.ds(r0, BO)]
            ae = ae * (1.0 / ae[20:21, :])
            ao = ao * (1.0 / ao[0:1, :])
            pieces.append(ae[0:16, :])
            pieces.append(jnp.where(row8 < 4, ae[16:24, :], ao[0:8, :]))
            pieces.append(ao[8:24, :])
        ot = jnp.concatenate(pieces, axis=0)
        o = ot.T.astype(jnp.bfloat16)
        a = jnp.dot(o, wo_ref[...], preferred_element_type=jnp.float32)

        hh = jnp.dot(xq, w1_ref[...], preferred_element_type=jnp.float32)
        hh = jnp.maximum(hh, 0.0).astype(jnp.bfloat16)
        b = jnp.dot(hh, w2_ref[...], preferred_element_type=jnp.float32)

        z = jnp.sum(xq.astype(jnp.float32) * gw_ref[...].astype(jnp.float32), axis=-1, keepdims=True)
        g = jax.nn.sigmoid(z)
        o_ref[...] = (g * a + (1.0 - g) * b).astype(o_ref.dtype)

    def call(A_x, A_wqkv, A_wo, B_x, B_w1, B_w2, gate_w):
        x = A_x.reshape(S, D)
        gw = gate_w.reshape(1, D)
        full = lambda shp: pl.BlockSpec(shp, lambda i: (0,) * len(shp))
        out = pl.pallas_call(
            kernel,
            grid=(NO,),
            in_specs=[full((S, D)), full((D, 3 * D)), full((D, D)), full((D, DFF)), full((DFF, D)), full((1, D))],
            out_specs=pl.BlockSpec((BO, D), lambda i: (i, 0)),
            out_shape=jax.ShapeDtypeStruct((S, D), jnp.bfloat16),
            scratch_shapes=[
                pltpu.VMEM((NWIN, S, 128), jnp.bfloat16),
                pltpu.VMEM((H, VROWS, S), jnp.float32),
                pltpu.VMEM((NWIN, S, 128), jnp.float32),
                pltpu.VMEM((H, VROWS, S), jnp.float32),
                pltpu.VMEM((S, BQ), jnp.float32),
                pltpu.VMEM((S, BQ), jnp.float32),
                pltpu.VMEM((8, BQ), jnp.float32),
                pltpu.VMEM((8, BQ), jnp.float32),
            ],
            compiler_params=pltpu.CompilerParams(
                dimension_semantics=("arbitrary",),
                vmem_limit_bytes=100 * 1024 * 1024),
        )(x, A_wqkv, A_wo, B_w1, B_w2, gw)
        return out.reshape(1, S, D)
    return call


_call = make_kernel()


@jax.jit
def pallas_gated_mix__softmax_full_mha__dense_activation_relu__prompt_kernel(
    A_x: jax.Array,
    A_wqkv: jax.Array,
    A_wo: jax.Array,
    B_x: jax.Array,
    B_w1: jax.Array,
    B_w2: jax.Array,
    gate_w: jax.Array,
):
    return _call(A_x, A_wqkv, A_wo, B_x, B_w1, B_w2, gate_w)
```

```python
import math
import jax
import jax.numpy as jnp
from jax import lax
import jax.experimental.pallas as pl
import jax.experimental.pallas.tpu as pltpu

S = 2048
D = 640
H = 32
DH = 20
DFF = 1536
NWIN = 6
VROWS = 24
KC = 128
NC = S // KC
BQ = 512
NQ = S // BQ
NJ = BQ // 128
NCT = S // 128
NSTEP = NQ * NC

NN = (((1,), (0,)), ((), ()))
TN = (((0,), (1,)), ((), ()))
F32 = jnp.float32
BF16 = jnp.bfloat16
U32 = jnp.uint32


def _window(a, w):
    c0 = 120 * w
    g0 = c0 // 128
    g1 = min(c0 + 119, D - 1) // 128
    lo = a[:, g0 * 128:(g0 + 1) * 128]
    if g1 == g0:
        return lo
    lane = lax.broadcasted_iota(jnp.int32, lo.shape, 1)
    return jnp.where(lane >= (c0 % 128), lo, a[:, g1 * 128:(g1 + 1) * 128])


def make_kernel(RA=512, RB=512, BO=256, KV=16, SK=2, NSLOT=8, NIT=None, FORCE_FALLBACK=False,
                AH=1, PEND=60, NACC=2, LEAD=3, NR=4, INSTAT=False, VFLAT=False):
    NO = S // BO
    NRA = S // RA
    NRB = S // RB
    qscale = (DH ** -0.5) * math.log2(math.e)
    KM = KC - KV
    GV = KV // 8

    def kernel(x_hbm, wqkv_hbm, wo_hbm, w1_hbm, w2_hbm, gw_ref, o_ref,
               x_ref, wqkv_ref, wo_ref, w1_ref, w2_ref, sems,
               kh_ref, vt_ref, qh_ref, qt_ref, koff_ref, qba_ref, qbb_ref, pb_ref, ot_ref, st_ref, *kb_refs):
        i = pl.program_id(0)
        qb_refs = (qba_ref, qbb_ref)

        def x_copy(c):
            r = pl.multiple_of(c * RA, RA)
            return pltpu.make_async_copy(x_hbm.at[pl.ds(r, RA), :], x_ref.at[pl.ds(r, RA), :], sems.at[c])

        def w_copy(j):
            return pltpu.make_async_copy(wqkv_hbm.at[:, pl.ds(j * D, D)], wqkv_ref.at[:, pl.ds(j * D, D)],
                                         sems.at[NRA + j])

        def late_copies():
            return [pltpu.make_async_copy(wo_hbm, wo_ref, sems.at[NRA + 3]),
                    pltpu.make_async_copy(w1_hbm, w1_ref, sems.at[NRA + 4]),
                    pltpu.make_async_copy(w2_hbm, w2_ref, sems.at[NRA + 5])]

        @pl.when(i == 0)
        def _():
            w_copy(0).start()
            x_copy(0).start()
            w_copy(0).wait()
            for c in range(1, NRA):
                x_copy(c).start()
            w_copy(1).start()
            w_copy(2).start()
            for cp in late_copies():
                cp.start()

            def proj_q(c, carry):
                r0 = pl.multiple_of(c * RA, RA)
                x_copy(c).wait()
                xc = x_ref[pl.ds(r0, RA), :]
                qt = lax.dot_general(wqkv_ref[:, 0:D], xc, TN, preferred_element_type=F32) * qscale
                qt = qt.astype(BF16).astype(F32)
                zpad = jnp.zeros((32 - DH, RA), F32)
                for h in range(H):
                    rows = qt[DH * h:DH * h + DH, :]
                    qh_ref[h, :, pl.ds(r0, RA)] = pltpu.bitcast(
                        jnp.concatenate([rows, zpad], axis=0).astype(BF16), U32)
                    if KV:
                        qt_ref[h, 0:DH, pl.ds(r0, RA)] = rows
                return carry
            lax.fori_loop(0, NRA, proj_q, 0)
            w_copy(1).wait()
            w_copy(2).wait()

            def proj_v(r0, n):
                xc = x_ref[pl.ds(r0, n), :]
                vt = lax.dot_general(wqkv_ref[:, 2 * D:3 * D], xc, TN, preferred_element_type=F32)
                row = lax.broadcasted_iota(jnp.int32, (VROWS, n), 0)
                for h in range(H):
                    st = (DH * h) // 8 * 8
                    off = DH * h - st
                    blk = vt[st:st + VROWS, :]
                    vt_ref[h, :, pl.ds(r0, n)] = jnp.where((row >= off) & (row < off + DH), blk, 1.0)

            def proj_kv(c, carry):
                r0 = pl.multiple_of(c * RB, RB)
                xc = x_ref[pl.ds(r0, RB), :]
                k = jnp.dot(xc, wqkv_ref[:, D:2 * D], preferred_element_type=F32).astype(BF16).astype(F32)
                r0h = pl.multiple_of(c * (RB // 2), RB // 2)
                no = RB // KC * KV
                for w in range(NWIN):
                    kwin = _window(k, w)
                    kpk = pltpu.bitcast(kwin.astype(BF16), U32)
                    if KV:
                        ko = jnp.concatenate([kwin[b * KC + KM:(b + 1) * KC, :] for b in range(RB // KC)], axis=0)
                    for h in range(6 * w, min(6 * w + 6, H)):
                        off = (DH * h) % 128
                        kh_ref[h, pl.ds(r0h, RB // 2), :] = pltpu.roll(kpk, 128 - off, 1) if off else kpk
                        if KV:
                            koff_ref[h, pl.ds(pl.multiple_of(c * no, no), no), :] = (
                                pltpu.roll(ko, 128 - off, 1) if off else ko)
                proj_v(r0, RB)
                return carry
            lax.fori_loop(0, NRB, proj_kv, 0)

            fmask = lax.broadcasted_iota(jnp.int32, (8, 128), 1) < (i - 1)

            def tied(v, tie):
                return v if tie is None else jnp.where(fmask, tie, v)

            def part(n, k, nsteps):
                return range((k * n) // nsteps, ((k + 1) * n) // nsteps) if k < nsteps else range(0)

            def prep_qb(hh, par, k, nsteps, tie=None):
                for e in part(DH * NCT, k, nsteps):
                    ct, d = e // DH, e % DH
                    qb_refs[par][0, d, :, ct * 128:(ct + 1) * 128] = tied(jnp.broadcast_to(
                        qt_ref[hh, d:d + 1, ct * 128:(ct + 1) * 128], (8, 128)), tie)

            def prep_kb(hh, c, k, nsteps, tie=None):
                kv = {}
                for e in part(GV * DH, k, nsteps):
                    g, d = e // DH, e % DH
                    if g not in kv:
                        kv[g] = tied(koff_ref[hh, 8 * (c * GV + g):8 * (c * GV + g) + 8, :], tie)
                    kb_refs[c % NR][0, g, d] = jnp.broadcast_to(kv[g][:, d:d + 1], (8, 128))

            def pieces(par, k, zbase, last):
                c, qb = k // NQ, k % NQ
                slot = k % NSLOT
                for jj in range(NJ):
                    zk = 0 if zbase is None else i * (NSTEP + 1 + zbase * NJ + jj)
                    cols = slice(qb * BQ + jj * 128, qb * BQ + (jj + 1) * 128)
                    accs = {}
                    for d in range(DH):
                        qv = qb_refs[par][zk, d, :, cols]
                        for g in range(GV):
                            term = kb_refs[c % NR][zk, g, d] * qv
                            if d == 0 and last is not None:
                                r = (jj * (KM // 8)) // NJ
                                term = tied(term, last[8 * r:8 * r + 8, jj * 128:(jj + 1) * 128])
                            key = (g, d % NACC)
                            accs[key] = term if key not in accs else accs[key] + term
                    for g in range(GV):
                        al = [accs[(g, n_)] for n_ in range(NACC)]
                        while len(al) > 1:
                            al = [al[2 * n_] + al[2 * n_ + 1] if 2 * n_ + 1 < len(al) else al[2 * n_]
                                  for n_ in range((len(al) + 1) // 2)]
                        pb_ref[slot, KM + 8 * g:KM + 8 * g + 8, jj * 128:(jj + 1) * 128] = jnp.exp2(al[0])

            def do_pv(h, par, kk):
                c, qb = kk // NQ, kk % NQ
                p = pb_ref[kk % NSLOT].astype(BF16)
                r = lax.dot_general(vt_ref[h, :, c * KC:(c + 1) * KC], p, NN, preferred_element_type=F32)
                if c > 0:
                    r = r + ot_ref[h, :, qb * BQ:(qb + 1) * BQ]
                ot_ref[h, :, qb * BQ:(qb + 1) * BQ] = r
                if INSTAT and c == NC - 1:
                    a = jnp.abs(r)
                    mx = jnp.maximum(jnp.maximum(a[:, 0:128], a[:, 128:256]), jnp.maximum(a[:, 256:384], a[:, 384:512]))
                    st_ref[par, 0:VROWS, :] = jnp.maximum(st_ref[par, 0:VROWS, :], mx)
                    lr = r[16:24, :] if par == 0 else r[0:8, :]
                    mn = jnp.minimum(jnp.minimum(lr[:, 0:128], lr[:, 128:256]), jnp.minimum(lr[:, 256:384], lr[:, 384:512]))
                    st_ref[par, VROWS:VROWS + 8, :] = jnp.minimum(st_ref[par, VROWS:VROWS + 8, :], mn)

            if KV:
                prep_qb(0, 0, 0, 1)
                for c_ in range(LEAD):
                    prep_kb(0, c_, 0, 1)
            for k in range(NSTEP - SK, NSTEP):
                pb_ref[k % NSLOT] = jnp.ones((KC, BQ), F32)
                qb_ = k % NQ
                ot_ref[1, :, qb_ * BQ:(qb_ + 1) * BQ] = jnp.zeros((VROWS, BQ), F32)
            if INSTAT:
                st_ref[:, 0:VROWS, :] = jnp.zeros((2, VROWS, 128), F32)
                st_ref[:, VROWS:VROWS + 8, :] = jnp.ones((2, 8, 128), F32)
            if KV:
                for k in range(AH):
                    pieces(0, k, None, None)

            def body(u, carry):
                last = None
                for par in range(2):
                    h = 2 * u + par
                    hn = h + 1 if par == 0 else jnp.minimum(h + 1, H - 1)
                    hp = h - 1 if par == 1 else jnp.maximum(h - 1, 1)
                    for k in range(NSTEP):
                        c, qb = k // NQ, k % NQ
                        zk = i * (k + 1)
                        kl = pltpu.bitcast(kh_ref[h, c * KC // 2:(c * KC + KM) // 2, :], BF16)[:, 0:32]
                        qm = pltpu.bitcast(qh_ref[h + zk, :, qb * BQ:(qb + 1) * BQ], BF16)
                        s = lax.dot_general(kl, qm, NN, preferred_element_type=F32)
                        pb_ref[k % NSLOT, 0:KM, :] = jnp.exp2(s)
                        if KV:
                            if k + AH < NSTEP:
                                pieces(par, k + AH, k, last)
                            else:
                                pieces(1 - par, k + AH - NSTEP, k, last)
                            prep_qb(hn, 1 - par, k, PEND, None if last is None else last[0:8, 0:128])
                            tie = None if last is None else last[8:16, 0:128]
                            if c + LEAD < NC:
                                prep_kb(h, c + LEAD, qb, NQ, tie)
                            else:
                                prep_kb(hn, c + LEAD - NC, qb, NQ, tie)
                        last = s
                        if k >= SK:
                            do_pv(h, par, k - SK)
                        else:
                            do_pv(hp, 1 - par, NSTEP + k - SK)
                return carry

            lax.fori_loop(0, H // 2 if NIT is None else NIT, body, 0)
            for k in range(SK):
                do_pv(H - 1, 1, NSTEP + k - SK)

            if INSTAT:
                arow = lax.broadcasted_iota(jnp.int32, (VROWS, 128), 0)
                lrow = lax.broadcasted_iota(jnp.int32, (8, 128), 0)
                bad = jnp.zeros((8, 128), F32)
                for par in range(2):
                    is_l = (arow < 4 * par) | (arow >= 4 * par + DH)
                    hi = jnp.where(is_l, 2.0 ** 60, 2.0 ** 100)
                    v = jnp.where(st_ref[par, 0:VROWS, :] <= hi, 0.0, 1.0)
                    bad = bad + v[0:8] + v[8:16] + v[16:24]
                    is_l8 = (lrow >= 4) if par == 0 else (lrow < 4)
                    bad = bad + jnp.where(is_l8, jnp.where(st_ref[par, VROWS:VROWS + 8, :] >= 2.0 ** -30, 0.0, 1.0), 0.0)
            else:
                arow = lax.broadcasted_iota(jnp.int32, (VROWS, BQ), 0)

                def check(t, bad):
                    for par in range(2):
                        is_l = (arow < 4 * par) | (arow >= 4 * par + DH)
                        lo = jnp.where(is_l, 2.0 ** -30, -(2.0 ** 100))
                        hi = jnp.where(is_l, 2.0 ** 60, 2.0 ** 100)
                        for qb in range(NQ):
                            a = ot_ref[2 * t + par, :, qb * BQ:(qb + 1) * BQ]
                            bad = bad + jnp.where((a >= lo) & (a <= hi), 0.0, 1.0)
                    return bad
                bad = lax.fori_loop(0, H // 2, check, jnp.zeros((VROWS, BQ), F32))
            nbad = jnp.sum(bad)

            @pl.when((nbad > 0.0) | FORCE_FALLBACK)
            def _():
                def item(t, carry):
                    h = lax.shift_right_logical(t, 2)
                    q0 = pl.multiple_of(lax.bitwise_and(t, NQ - 1) * BQ, BQ)
                    qm = pltpu.bitcast(qh_ref[h, :, pl.ds(q0, BQ)], BF16)

                    def chunk(c, st):
                        m, acc = st
                        kl = pltpu.bitcast(
                            kh_ref[h, pl.ds(pl.multiple_of(c * (KC // 2), KC // 2), KC // 2), :], BF16)[:, 0:32]
                        s = lax.dot_general(kl, qm, NN, preferred_element_type=F32)
                        m_new = jnp.maximum(m, jnp.max(s, axis=0, keepdims=True))
                        p = jnp.exp2(s - m_new).astype(BF16)
                        r = lax.dot_general(vt_ref[h, :, pl.ds(pl.multiple_of(c * KC, KC), KC)], p, NN,
                                            preferred_element_type=F32)
                        return m_new, acc * jnp.exp2(m - m_new) + r

                    m0 = jnp.full((1, BQ), -jnp.inf, F32)
                    _, acc = lax.fori_loop(0, NC, chunk, (m0, jnp.zeros((VROWS, BQ), F32)))
                    ot_ref[h, :, pl.ds(q0, BQ)] = acc
                    return carry
                lax.fori_loop(0, H * NQ, item, 0)

            for cp in late_copies():
                cp.wait()

        r0 = pl.multiple_of(i * BO, BO)
        xq = x_ref[pl.ds(r0, BO), :]

        hh = jnp.dot(xq, w1_ref[...], preferred_element_type=F32)
        hh = jnp.maximum(hh, 0.0).astype(BF16)
        b = jnp.dot(hh, w2_ref[...], preferred_element_type=F32)

        row8 = lax.broadcasted_iota(jnp.int32, (8, BO), 0)
        blocks = []
        for pair in range(H // 2):
            ae = ot_ref[2 * pair, :, pl.ds(r0, BO)]
            ao = ot_ref[2 * pair + 1, :, pl.ds(r0, BO)]
            ae = ae * (1.0 / ae[20:21, :])
            ao = ao * (1.0 / ao[0:1, :])
            blocks.append(ae[0:16, :])
            blocks.append(jnp.where(row8 < 4, ae[16:24, :], ao[0:8, :]))
            blocks.append(ao[8:24, :])
        o = jnp.concatenate(blocks, axis=0).T.astype(BF16)
        a = jnp.dot(o, wo_ref[...], preferred_element_type=F32)

        z = jnp.sum(xq.astype(F32) * gw_ref[...].astype(F32), axis=-1, keepdims=True)
        g = jax.nn.sigmoid(z)
        o_ref[...] = (g * a + (1.0 - g) * b).astype(o_ref.dtype)

    def call(A_x, A_wqkv, A_wo, B_x, B_w1, B_w2, gate_w):
        x = A_x.reshape(S, D)
        gw = gate_w.reshape(1, D)
        anyspec = pl.BlockSpec(memory_space=pl.ANY)
        out = pl.pallas_call(
            kernel,
            grid=(NO,),
            in_specs=[anyspec, anyspec, anyspec, anyspec, anyspec, pl.BlockSpec((1, D), lambda i: (0, 0))],
            out_specs=pl.BlockSpec((BO, D), lambda i: (i, 0)),
            out_shape=jax.ShapeDtypeStruct((S, D), BF16),
            scratch_shapes=[
                pltpu.VMEM((S, D), BF16),
                pltpu.VMEM((D, 3 * D), BF16),
                pltpu.VMEM((D, D), BF16),
                pltpu.VMEM((D, DFF), BF16),
                pltpu.VMEM((DFF, D), BF16),
                pltpu.SemaphoreType.DMA((NRA + 6,)),
                pltpu.VMEM((H, S // 2, 128), U32),
                pltpu.VMEM((H, VROWS, S), F32),
                pltpu.VMEM((H, 16, S), U32),
                pltpu.VMEM((H, VROWS, S), F32),
                pltpu.VMEM((H, NC * max(KV, 8), 128), F32),
                pltpu.VMEM((1, DH, 8, S), F32),
                pltpu.VMEM((1, DH, 8, S), F32),
                pltpu.VMEM((NSLOT, KC, BQ), F32),
                pltpu.VMEM((H, VROWS, S), F32),
                pltpu.VMEM((2, VROWS + 8, 128), F32),
            ] + [pltpu.VMEM((1, max(GV, 1), DH, 8, 128), F32) for _ in range(NR)],
            compiler_params=pltpu.CompilerParams(
                dimension_semantics=("arbitrary",),
                vmem_limit_bytes=100 * 1024 * 1024),
        )(x, A_wqkv, A_wo, B_w1, B_w2, gw)
        return out.reshape(1, S, D)
    return call


_call = make_kernel(INSTAT=True)


@jax.jit
def pallas_gated_mix__softmax_full_mha__dense_activation_relu__prompt_kernel(
    A_x: jax.Array,
    A_wqkv: jax.Array,
    A_wo: jax.Array,
    B_x: jax.Array,
    B_w1: jax.Array,
    B_w2: jax.Array,
    gate_w: jax.Array,
):
    return _call(A_x, A_wqkv, A_wo, B_x, B_w1, B_w2, gate_w)
```

```python
import math
import jax
import jax.numpy as jnp
from jax import lax
import jax.experimental.pallas as pl
import jax.experimental.pallas.tpu as pltpu

S = 2048
D = 640
H = 32
DH = 20
DFF = 1536
NWIN = 6
VROWS = 24
KC = 128
KV = 16
KM = KC - KV
GV = KV // 8
NC = S // KC
BQ = 512
NQ = S // BQ
NJ = BQ // 128
NCT = S // 128
NSTEP = NQ * NC

NN = (((1,), (0,)), ((), ()))
TN = (((0,), (1,)), ((), ()))
F32 = jnp.float32
BF16 = jnp.bfloat16
U32 = jnp.uint32


def _window(a, w):
    c0 = 120 * w
    g0 = c0 // 128
    g1 = min(c0 + 119, D - 1) // 128
    lo = a[:, g0 * 128:(g0 + 1) * 128]
    if g1 == g0:
        return lo
    lane = lax.broadcasted_iota(jnp.int32, lo.shape, 1)
    return jnp.where(lane >= (c0 % 128), lo, a[:, g1 * 128:(g1 + 1) * 128])


def _part(n, k, nsteps):
    return range((k * n) // nsteps, ((k + 1) * n) // nsteps) if k < nsteps else range(0)


def make_kernel(RA=512, RB=512, BO=256, SK=2, NSLOT=8, AH=1, PEND=60, LEAD=3, NR=4, JB=2,
                TDS=(5, 15), TR=(3, 6, 10, 13), ER=(2, 5, 8, 11), PR=(8, 8), HB=2,
                NIT=None, FORCE_FALLBACK=False, G1D=True, WQT=True):
    NO = S // BO
    NRA = S // RA
    NRB = S // RB
    qscale = (DH ** -0.5) * math.log2(math.e)

    def kernel(x_hbm, wqkv_hbm, wo_hbm, w1_hbm, w2_hbm, gw_hbm, o_ref,
               x_ref, wqkv_ref, wo_ref, w1_ref, w2_ref, gw_ref, sems,
               kh_ref, vt_ref, qh_ref, qt_ref, koff_ref, qba_ref, qbb_ref, pb_ref, ot_ref, st_ref, wqt_ref, *kb_refs):
        i = pl.program_id(0)
        qb_refs = (qba_ref, qbb_ref)

        def x_copy(c):
            r = pl.multiple_of(c * RA, RA)
            return pltpu.make_async_copy(x_hbm.at[pl.ds(r, RA), :], x_ref.at[pl.ds(r, RA), :], sems.at[c])

        def w_copy(j):
            return pltpu.make_async_copy(wqkv_hbm.at[:, pl.ds(j * D, D)], wqkv_ref.at[:, pl.ds(j * D, D)],
                                         sems.at[NRA + j])

        def late_copies():
            return [pltpu.make_async_copy(wo_hbm, wo_ref, sems.at[NRA + 3]),
                    pltpu.make_async_copy(w1_hbm, w1_ref, sems.at[NRA + 4]),
                    pltpu.make_async_copy(w2_hbm, w2_ref, sems.at[NRA + 5]),
                    pltpu.make_async_copy(gw_hbm, gw_ref, sems.at[NRA + 6])]

        @pl.when(i == 0)
        def _():
            w_copy(0).start()
            x_copy(0).start()
            for k in range(NSTEP - SK, NSTEP):
                pb_ref[k % NSLOT] = jnp.ones((KC, BQ), F32)
                ot_ref[1, :, (k % NQ) * BQ:(k % NQ + 1) * BQ] = jnp.zeros((VROWS, BQ), F32)
            st_ref[:, 0:VROWS, :] = jnp.zeros((2, VROWS, 128), F32)
            st_ref[:, VROWS:VROWS + 8, :] = jnp.ones((2, 8, 128), F32)
            w_copy(0).wait()
            for c in range(1, NRA):
                x_copy(c).start()
            w_copy(1).start()
            w_copy(2).start()
            for cp in late_copies():
                cp.start()
            if WQT:
                wqt_ref[...] = wqkv_ref[:, 0:D].T

            def proj_q(c, carry):
                r0 = pl.multiple_of(c * RA, RA)
                x_copy(c).wait()
                xc = x_ref[pl.ds(r0, RA), :]
                if WQT:
                    qt = lax.dot_general(wqt_ref[...], xc, (((1,), (1,)), ((), ())), preferred_element_type=F32) * qscale
                else:
                    qt = lax.dot_general(wqkv_ref[:, 0:D], xc, TN, preferred_element_type=F32) * qscale
                qt = qt.astype(BF16).astype(F32)
                zpad = jnp.zeros((32 - DH, RA), F32)
                for h in range(H):
                    rows = qt[DH * h:DH * h + DH, :]
                    qh_ref[h, :, pl.ds(r0, RA)] = pltpu.bitcast(
                        jnp.concatenate([rows, zpad], axis=0).astype(BF16), U32)
                    qt_ref[h, 0:DH, pl.ds(r0, RA)] = rows
                return carry
            lax.fori_loop(0, NRA, proj_q, 0)
            w_copy(1).wait()
            w_copy(2).wait()

            def proj_kv(c, carry):
                r0 = pl.multiple_of(c * RB, RB)
                xc = x_ref[pl.ds(r0, RB), :]
                k = jnp.dot(xc, wqkv_ref[:, D:2 * D], preferred_element_type=F32).astype(BF16).astype(F32)
                r0h = pl.multiple_of(c * (RB // 2), RB // 2)
                no = RB // KC * KV
                for w in range(NWIN):
                    kwin = _window(k, w)
                    kpk = pltpu.bitcast(kwin.astype(BF16), U32)
                    ko = jnp.concatenate([kwin[b * KC + KM:(b + 1) * KC, :] for b in range(RB // KC)], axis=0)
                    for h in range(6 * w, min(6 * w + 6, H)):
                        off = (DH * h) % 128
                        kh_ref[h, pl.ds(r0h, RB // 2), :] = pltpu.roll(kpk, 128 - off, 1) if off else kpk
                        koff_ref[h, pl.ds(pl.multiple_of(c * no, no), no), :] = (
                            pltpu.roll(ko, 128 - off, 1) if off else ko)
                vt = lax.dot_general(wqkv_ref[:, 2 * D:3 * D], xc, TN, preferred_element_type=F32)
                row = lax.broadcasted_iota(jnp.int32, (VROWS, RB), 0)
                for h in range(H):
                    st = (DH * h) // 8 * 8
                    off = DH * h - st
                    blk = vt[st:st + VROWS, :]
                    vt_ref[h, :, pl.ds(r0, RB)] = jnp.where((row >= off) & (row < off + DH), blk, 1.0)
                return carry
            lax.fori_loop(0, NRB, proj_kv, 0)

            fmask = lax.broadcasted_iota(jnp.int32, (8, 128), 1) < (i - 1)

            def tied(v, tie):
                return v if tie is None else jnp.where(fmask, tie, v)

            def rows_of(s, r, jj=0):
                return None if s is None else s[8 * r:8 * r + 8, jj * 128:(jj + 1) * 128]

            def prep_qb(hh, par, k, nsteps, tie=None):
                for e in _part(DH * NCT, k, nsteps):
                    ct, d = e // DH, e % DH
                    qb_refs[par][0, ct, d] = tied(jnp.broadcast_to(
                        qt_ref[hh, d:d + 1, ct * 128:(ct + 1) * 128], (8, 128)), tie)

            def prep_kb(hh, c, k, nsteps, tie=None):
                kv = {}
                for e in _part(GV * DH, k, nsteps):
                    g, d = e % GV, e // GV
                    if g not in kv:
                        kv[g] = tied(koff_ref[hh, 8 * (c * GV + g):8 * (c * GV + g) + 8, :], tie)
                    kb_refs[c % NR][0, g, d] = jnp.broadcast_to(kv[g][:, d:d + 1], (8, 128))

            def vpu_scores(par, k, zbase, last, tr):
                c, qb = k // NQ, k % NQ
                for j0 in range(0, NJ, JB):
                    zk = 0 if zbase is None else i * (NSTEP + 1 + zbase * NJ + j0)
                    acc = {}
                    for d in range(DH):
                        kbs = [kb_refs[c % NR][zk, g, d] for g in range(GV)]
                        for jj in range(j0, j0 + JB):
                            qv = qb_refs[par][zk, qb * NJ + jj, d]
                            for g in range(GV):
                                term = kbs[g] * qv
                                if d in TDS:
                                    term = tied(term, rows_of(last, tr[(j0 // JB) * len(TDS) + TDS.index(d)], jj))
                                acc[g, jj] = term if d == 0 else acc[g, jj] + term
                    for jj in range(j0, j0 + JB):
                        for g in range(GV):
                            pb_ref[k % NSLOT, KM + 8 * g:KM + 8 * g + 8, jj * 128:(jj + 1) * 128] = (
                                jnp.exp2(acc[g, jj]))

            def do_pv(h, par, kk):
                c, qb = kk // NQ, kk % NQ
                p = pb_ref[kk % NSLOT].astype(BF16)
                r = lax.dot_general(vt_ref[h, :, c * KC:(c + 1) * KC], p, NN, preferred_element_type=F32)
                if c > 0:
                    r = r + ot_ref[h, :, qb * BQ:(qb + 1) * BQ]
                ot_ref[h, :, qb * BQ:(qb + 1) * BQ] = r
                if c == NC - 1:
                    a = jnp.abs(r)
                    mx = jnp.maximum(jnp.maximum(a[:, 0:128], a[:, 128:256]),
                                     jnp.maximum(a[:, 256:384], a[:, 384:512]))
                    st_ref[par, 0:VROWS, :] = jnp.maximum(st_ref[par, 0:VROWS, :], mx)
                    lr = r[16:24, :] if par == 0 else r[0:8, :]
                    mn = jnp.minimum(jnp.minimum(lr[:, 0:128], lr[:, 128:256]),
                                     jnp.minimum(lr[:, 256:384], lr[:, 384:512]))
                    st_ref[par, VROWS:VROWS + 8, :] = jnp.minimum(st_ref[par, VROWS:VROWS + 8, :], mn)

            prep_qb(0, 0, 0, 1)
            for c_ in range(LEAD):
                prep_kb(0, c_, 0, 1)
            for k in range(AH + 1):
                vpu_scores(0, k, None, None, TR)

            def body(u, carry):
                last = None
                for hb in range(HB):
                    par = hb % 2
                    h = HB * u + hb
                    hn = h + 1 if hb < HB - 1 else jnp.minimum(h + 1, H - 1)
                    hp = h - 1 if hb > 0 else jnp.maximum(h - 1, 1)
                    for k in range(NSTEP):
                        c, qb = k // NQ, k % NQ
                        zb = (hb // 2) * NSTEP + k
                        kl = pltpu.bitcast(kh_ref[h, c * KC // 2:(c * KC + KM) // 2, :], BF16)[:, 0:32]
                        qm = pltpu.bitcast(qh_ref[h + i * (k + 1), :, qb * BQ:(qb + 1) * BQ], BF16)
                        s = lax.dot_general(kl, qm, NN, preferred_element_type=F32)
                        pb_ref[k % NSLOT, 0:KM, :] = jnp.exp2(s)
                        if last is None:
                            pass
                        elif k + AH < NSTEP:
                            vpu_scores(par, k + AH, zb, last, TR)
                        else:
                            vpu_scores(1 - par, k + AH - NSTEP, zb, last, TR)
                        prep_qb(hn, 1 - par, k, PEND, rows_of(last, PR[0]))
                        if c + LEAD < NC:
                            prep_kb(h, c + LEAD, qb, NQ, rows_of(last, PR[1]))
                        else:
                            prep_kb(hn, c + LEAD - NC, qb, NQ, rows_of(last, PR[1]))
                        if k >= SK:
                            do_pv(h, par, k - SK)
                        else:
                            do_pv(hp, 1 - par, NSTEP + k - SK)
                        last = s
                vpu_scores(0, AH, NSTEP * 20, last, ER)
                return carry

            lax.fori_loop(0, H // HB if NIT is None else NIT, body, 0)
            for k in range(SK):
                do_pv(H - 1, 1, NSTEP + k - SK)

            arow = lax.broadcasted_iota(jnp.int32, (VROWS, 128), 0)
            lrow = lax.broadcasted_iota(jnp.int32, (8, 128), 0)
            bad = jnp.zeros((8, 128), F32)
            for par in range(2):
                is_l = (arow < 4 * par) | (arow >= 4 * par + DH)
                hi = jnp.where(is_l, 2.0 ** 60, 2.0 ** 100)
                v = jnp.where(st_ref[par, 0:VROWS, :] <= hi, 0.0, 1.0)
                bad = bad + v[0:8] + v[8:16] + v[16:24]
                is_l8 = (lrow >= 4) if par == 0 else (lrow < 4)
                low = jnp.where(st_ref[par, VROWS:VROWS + 8, :] >= 2.0 ** -30, 0.0, 1.0)
                bad = bad + jnp.where(is_l8, low, 0.0)
            nbad = jnp.sum(bad)

            @pl.when((nbad > 0.0) | FORCE_FALLBACK)
            def _():
                def item(t, carry):
                    h = lax.shift_right_logical(t, 2)
                    q0 = pl.multiple_of(lax.bitwise_and(t, NQ - 1) * BQ, BQ)
                    qm = pltpu.bitcast(qh_ref[h, :, pl.ds(q0, BQ)], BF16)

                    def chunk(c, st):
                        m, acc = st
                        kl = pltpu.bitcast(
                            kh_ref[h, pl.ds(pl.multiple_of(c * (KC // 2), KC // 2), KC // 2), :], BF16)[:, 0:32]
                        s = lax.dot_general(kl, qm, NN, preferred_element_type=F32)
                        m_new = jnp.maximum(m, jnp.max(s, axis=0, keepdims=True))
                        p = jnp.exp2(s - m_new).astype(BF16)
                        r = lax.dot_general(vt_ref[h, :, pl.ds(pl.multiple_of(c * KC, KC), KC)], p, NN,
                                            preferred_element_type=F32)
                        return m_new, acc * jnp.exp2(m - m_new) + r

                    m0 = jnp.full((1, BQ), -jnp.inf, F32)
                    _, acc = lax.fori_loop(0, NC, chunk, (m0, jnp.zeros((VROWS, BQ), F32)))
                    ot_ref[h, :, pl.ds(q0, BQ)] = acc
                    return carry
                lax.fori_loop(0, H * NQ, item, 0)

            for cp in late_copies():
                cp.wait()

        r0 = pl.multiple_of(i * BO, BO)
        xq = x_ref[pl.ds(r0, BO), :]

        hh = jnp.dot(xq, w1_ref[...], preferred_element_type=F32)
        hh = jnp.maximum(hh, 0.0).astype(BF16)
        b = jnp.dot(hh, w2_ref[...], preferred_element_type=F32)

        row8 = lax.broadcasted_iota(jnp.int32, (8, BO), 0)
        blocks = []
        for pair in range(H // 2):
            ae = ot_ref[2 * pair, :, pl.ds(r0, BO)]
            ao = ot_ref[2 * pair + 1, :, pl.ds(r0, BO)]
            ae = ae * (1.0 / ae[20:21, :])
            ao = ao * (1.0 / ao[0:1, :])
            blocks.append(ae[0:16, :])
            blocks.append(jnp.where(row8 < 4, ae[16:24, :], ao[0:8, :]))
            blocks.append(ao[8:24, :])
        o = jnp.concatenate(blocks, axis=0).T.astype(BF16)
        a = jnp.dot(o, wo_ref[...], preferred_element_type=F32)

        gw = gw_ref[...].astype(F32)
        if G1D:
            gw = gw.reshape(1, D)
        z = jnp.sum(xq.astype(F32) * gw, axis=-1, keepdims=True)
        g = jax.nn.sigmoid(z)
        o_ref[...] = (g * a + (1.0 - g) * b).astype(o_ref.dtype)

    def call(A_x, A_wqkv, A_wo, B_x, B_w1, B_w2, gate_w):
        x = A_x.reshape(S, D)
        anyspec = pl.BlockSpec(memory_space=pl.ANY)
        gw, gspec = (gate_w if G1D else gate_w.reshape(1, D)), anyspec
        out = pl.pallas_call(
            kernel,
            grid=(NO,),
            in_specs=[anyspec, anyspec, anyspec, anyspec, anyspec, gspec],
            out_specs=pl.BlockSpec((BO, D), lambda i: (i, 0)),
            out_shape=jax.ShapeDtypeStruct((S, D), BF16),
            scratch_shapes=[
                pltpu.VMEM((S, D), BF16),
                pltpu.VMEM((D, 3 * D), BF16),
                pltpu.VMEM((D, D), BF16),
                pltpu.VMEM((D, DFF), BF16),
                pltpu.VMEM((DFF, D), BF16),
                pltpu.VMEM((D,) if G1D else (1, D), BF16),
                pltpu.SemaphoreType.DMA((NRA + 7,)),
                pltpu.VMEM((H, S // 2, 128), U32),
                pltpu.VMEM((H, VROWS, S), F32),
                pltpu.VMEM((H, 16, S), U32),
                pltpu.VMEM((H, VROWS, S), F32),
                pltpu.VMEM((H, NC * KV, 128), F32),
                pltpu.VMEM((1, NCT, DH, 8, 128), F32),
                pltpu.VMEM((1, NCT, DH, 8, 128), F32),
                pltpu.VMEM((NSLOT, KC, BQ), F32),
                pltpu.VMEM((H, VROWS, S), F32),
                pltpu.VMEM((2, VROWS + 8, 128), F32),
                pltpu.VMEM((D, D), BF16),
            ] + [pltpu.VMEM((1, GV, DH, 8, 128), F32) for _ in range(NR)],
            compiler_params=pltpu.CompilerParams(
                dimension_semantics=("arbitrary",),
                vmem_limit_bytes=100 * 1024 * 1024),
        )(x, A_wqkv, A_wo, B_w1, B_w2, gw)
        return out.reshape(1, S, D)
    return call


_call = make_kernel()


@jax.jit
def pallas_gated_mix__softmax_full_mha__dense_activation_relu__prompt_kernel(
    A_x: jax.Array,
    A_wqkv: jax.Array,
    A_wo: jax.Array,
    B_x: jax.Array,
    B_w1: jax.Array,
    B_w2: jax.Array,
    gate_w: jax.Array,
):
    return _call(A_x, A_wqkv, A_wo, B_x, B_w1, B_w2, gate_w)
```

```python
import math

import jax
import jax.numpy as jnp
from jax import lax
import jax.experimental.pallas as pl
import jax.experimental.pallas.tpu as pltpu

S = 2048
D = 640
H = 32
DH = 20
DFF = 1536

NWIN = 6
VROWS = 24
KC = 128
KV = 16
KM = KC - KV
GV = KV // 8
NC = S // KC
BQ = 512
NQ = S // BQ
NJ = BQ // 128
NCT = S // 128
NSTEP = NQ * NC
JB = 2

RA = 512
RB = 512
BO = 256
NRA, NRB, NO = S // RA, S // RB, S // BO

SK = 2
NSLOT = 8
AH = 1
LEAD = 2
NR = 4
PEND = 60
TDS = (5, 15)
TR = (3, 6, 10, 13)
ER = (2, 5, 8, 11)
PR = 8

QSCALE = (DH ** -0.5) * math.log2(math.e)

NN = (((1,), (0,)), ((), ()))
NT = (((1,), (1,)), ((), ()))
TN = (((0,), (1,)), ((), ()))
F32 = jnp.float32
BF16 = jnp.bfloat16
U32 = jnp.uint32


def _window(a, w):
    c0 = 120 * w
    g0 = c0 // 128
    g1 = min(c0 + 119, D - 1) // 128
    lo = a[:, g0 * 128:(g0 + 1) * 128]
    if g1 == g0:
        return lo
    lane = lax.broadcasted_iota(jnp.int32, lo.shape, 1)
    return jnp.where(lane >= (c0 % 128), lo, a[:, g1 * 128:(g1 + 1) * 128])


def _part(n, k, nsteps):
    return range((k * n) // nsteps, ((k + 1) * n) // nsteps) if k < nsteps else range(0)


def _kernel(x_hbm, wqkv_hbm, wo_hbm, w1_hbm, w2_hbm, gw_hbm, o_ref,
            x_ref, wqkv_ref, wo_ref, w1_ref, w2_ref, gw_ref, sems,
            wqt_ref, kh_ref, vt_ref, qh_ref, qt_ref, koff_ref, qba_ref, qbb_ref, pb_ref, ot_ref, st_ref,
            *kb_refs):
    i = pl.program_id(0)
    qb_refs = (qba_ref, qbb_ref)

    def x_copy(c):
        r = pl.multiple_of(c * RA, RA)
        return pltpu.make_async_copy(x_hbm.at[pl.ds(r, RA), :], x_ref.at[pl.ds(r, RA), :], sems.at[c])

    def w_copy(j):
        return pltpu.make_async_copy(wqkv_hbm.at[:, pl.ds(j * D, D)], wqkv_ref.at[:, pl.ds(j * D, D)],
                                     sems.at[NRA + j])

    def late_copies():
        return [pltpu.make_async_copy(wo_hbm, wo_ref, sems.at[NRA + 3]),
                pltpu.make_async_copy(w1_hbm, w1_ref, sems.at[NRA + 4]),
                pltpu.make_async_copy(w2_hbm, w2_ref, sems.at[NRA + 5]),
                pltpu.make_async_copy(gw_hbm, gw_ref, sems.at[NRA + 6])]

    @pl.when(i == 0)
    def _():
        w_copy(0).start()
        x_copy(0).start()
        for k in range(NSTEP - SK, NSTEP):
            pb_ref[k % NSLOT] = jnp.ones((KC, BQ), F32)
            ot_ref[1, :, (k % NQ) * BQ:(k % NQ + 1) * BQ] = jnp.zeros((VROWS, BQ), F32)
        st_ref[:, 0:VROWS, :] = jnp.zeros((2, VROWS, 128), F32)
        st_ref[:, VROWS:VROWS + 8, :] = jnp.ones((2, 8, 128), F32)
        w_copy(0).wait()
        for c in range(1, NRA):
            x_copy(c).start()
        w_copy(1).start()
        w_copy(2).start()
        for cp in late_copies():
            cp.start()
        wqt_ref[...] = wqkv_ref[:, 0:D].T

        def proj_q(c, carry):
            r0 = pl.multiple_of(c * RA, RA)
            x_copy(c).wait()
            xc = x_ref[pl.ds(r0, RA), :]
            qt = lax.dot_general(wqt_ref[...], xc, NT, preferred_element_type=F32) * QSCALE
            qt = qt.astype(BF16).astype(F32)
            zpad = jnp.zeros((32 - DH, RA), F32)
            for h in range(H):
                rows = qt[DH * h:DH * h + DH, :]
                qh_ref[h, :, pl.ds(r0, RA)] = pltpu.bitcast(
                    jnp.concatenate([rows, zpad], axis=0).astype(BF16), U32)
                qt_ref[h, 0:DH, pl.ds(r0, RA)] = rows
                if h == 0:
                    nb = RA // (JB * 128)
                    for b in range(nb):
                        for d in range(DH):
                            qba_ref[0, c * nb + b, d] = jnp.broadcast_to(
                                rows[d:d + 1, b * JB * 128:(b + 1) * JB * 128], (8, JB * 128))
            return carry
        lax.fori_loop(0, NRA, proj_q, 0)
        w_copy(1).wait()
        w_copy(2).wait()

        def proj_kv(c, carry):
            r0 = pl.multiple_of(c * RB, RB)
            xc = x_ref[pl.ds(r0, RB), :]
            k = jnp.dot(xc, wqkv_ref[:, D:2 * D], preferred_element_type=F32).astype(BF16).astype(F32)
            r0h = pl.multiple_of(c * (RB // 2), RB // 2)
            no = RB // KC * KV
            for w in range(NWIN):
                kwin = _window(k, w)
                kpk = pltpu.bitcast(kwin.astype(BF16), U32)
                ko = jnp.concatenate([kwin[b * KC + KM:(b + 1) * KC, :] for b in range(RB // KC)], axis=0)
                for h in range(6 * w, min(6 * w + 6, H)):
                    off = (DH * h) % 128
                    kh_ref[h, pl.ds(r0h, RB // 2), :] = pltpu.roll(kpk, 128 - off, 1) if off else kpk
                    koff_ref[h, pl.ds(pl.multiple_of(c * no, no), no), :] = (
                        pltpu.roll(ko, 128 - off, 1) if off else ko)
            vt = lax.dot_general(wqkv_ref[:, 2 * D:3 * D], xc, TN, preferred_element_type=F32)
            row = lax.broadcasted_iota(jnp.int32, (VROWS, RB), 0)
            for h in range(H):
                st = (DH * h) // 8 * 8
                off = DH * h - st
                blk = vt[st:st + VROWS, :]
                vt_ref[h, :, pl.ds(r0, RB)] = jnp.where((row >= off) & (row < off + DH), blk, 1.0)
            return carry
        lax.fori_loop(0, NRB, proj_kv, 0)

        fmask = lax.broadcasted_iota(jnp.int32, (8, 128), 1) < (i - 1)
        fmask2 = jnp.concatenate([fmask] * GV, axis=0)
        fmask3 = jnp.concatenate([fmask2] * JB, axis=1)

        def prep_qb(hh, par, k, tie):
            for e in _part(DH * NCT, k, PEND):
                ct, d = e // DH, e % DH
                v = jnp.broadcast_to(qt_ref[hh, d:d + 1, ct * 128:(ct + 1) * 128], (8, 128))
                if tie is not None:
                    v = jnp.where(fmask, tie, v)
                qb_refs[par][0, ct // JB, d, :, (ct % JB) * 128:(ct % JB + 1) * 128] = v

        def prep_kb(hh, c, k, nsteps, tie):
            kv = koff_ref[hh, c * KV:(c + 1) * KV, :]
            if tie is not None:
                kv = jnp.where(fmask2, jnp.concatenate([tie] * GV, axis=0), kv)
            for d in _part(DH, k, nsteps):
                kb_refs[c % NR][0, d] = jnp.broadcast_to(kv[:, d:d + 1], (KV, 128))

        def vpu_scores(par, k, zbase, last, tr):
            c, qb = k // NQ, k % NQ
            for j0 in range(0, NJ, JB):
                zk = 0 if zbase is None else i * (NSTEP + 1 + zbase * NJ + j0)
                kb = kb_refs[c % NR][zk]
                qv = qb_refs[par][zk, (qb * NJ + j0) // JB]
                terms = jnp.concatenate([kb] * JB, axis=2) * jnp.concatenate([qv] * GV, axis=1)
                if last is not None:
                    segs, d0 = [], 0
                    for n, d in enumerate(TDS):
                        r = tr[(j0 // JB) * len(TDS) + n]
                        tie = last[8 * r:8 * r + 8, j0 * 128:(j0 + JB) * 128]
                        segs.append(terms[d0:d])
                        segs.append(jnp.where(fmask3[None], jnp.concatenate([tie] * GV, axis=0)[None],
                                              terms[d:d + 1]))
                        d0 = d + 1
                    segs.append(terms[d0:DH])
                    terms = jnp.concatenate(segs, axis=0)
                pb_ref[k % NSLOT, KM:KC, j0 * 128:(j0 + JB) * 128] = jnp.exp2(jnp.sum(terms, axis=0))

        def do_pv(h, par, kk):
            c, qb = kk // NQ, kk % NQ
            p = pb_ref[kk % NSLOT].astype(BF16)
            r = lax.dot_general(vt_ref[h, :, c * KC:(c + 1) * KC], p, NN, preferred_element_type=F32)
            if c > 0:
                r = r + ot_ref[h, :, qb * BQ:(qb + 1) * BQ]
            ot_ref[h, :, qb * BQ:(qb + 1) * BQ] = r
            if c == NC - 1:
                a = jnp.abs(r)
                mx = jnp.maximum(jnp.maximum(a[:, 0:128], a[:, 128:256]),
                                 jnp.maximum(a[:, 256:384], a[:, 384:512]))
                st_ref[par, 0:VROWS, :] = jnp.maximum(st_ref[par, 0:VROWS, :], mx)
                lr = r[16:24, :] if par == 0 else r[0:8, :]
                mn = jnp.minimum(jnp.minimum(lr[:, 0:128], lr[:, 128:256]),
                                 jnp.minimum(lr[:, 256:384], lr[:, 384:512]))
                st_ref[par, VROWS:VROWS + 8, :] = jnp.minimum(st_ref[par, VROWS:VROWS + 8, :], mn)

        for c in range(LEAD):
            prep_kb(0, c, 0, 1, None)
        for k in range(AH + 1):
            vpu_scores(0, k, None, None, TR)

        def head_pair(u, carry):
            last = None
            for par in range(2):
                h = 2 * u + par
                hn = h + 1 if par == 0 else jnp.minimum(h + 1, H - 1)
                hp = h - 1 if par == 1 else jnp.maximum(h - 1, 1)
                for k in range(NSTEP):
                    c, qb = k // NQ, k % NQ
                    kl = pltpu.bitcast(kh_ref[h, c * KC // 2:(c * KC + KM) // 2, :], BF16)[:, 0:32]
                    qm = pltpu.bitcast(qh_ref[h + i * (k + 1), :, qb * BQ:(qb + 1) * BQ], BF16)
                    s = lax.dot_general(kl, qm, NN, preferred_element_type=F32)
                    pb_ref[k % NSLOT, 0:KM, :] = jnp.exp2(s)
                    if last is None:
                        pass
                    elif k + AH < NSTEP:
                        vpu_scores(par, k + AH, k, last, TR)
                    else:
                        vpu_scores(1 - par, k + AH - NSTEP, k, last, TR)
                    tie = None if last is None else last[8 * PR:8 * PR + 8, 0:128]
                    prep_qb(hn, 1 - par, k, tie)
                    if c + LEAD < NC:
                        prep_kb(h, c + LEAD, qb, NQ, tie)
                    else:
                        prep_kb(hn, c + LEAD - NC, qb, NQ, tie)
                    if k >= SK:
                        do_pv(h, par, k - SK)
                    else:
                        do_pv(hp, 1 - par, NSTEP + k - SK)
                    last = s
            vpu_scores(0, AH, NSTEP * 20, last, ER)
            return carry

        lax.fori_loop(0, H // 2, head_pair, 0)
        for k in range(SK):
            do_pv(H - 1, 1, NSTEP + k - SK)

        arow = lax.broadcasted_iota(jnp.int32, (VROWS, 128), 0)
        lrow = lax.broadcasted_iota(jnp.int32, (8, 128), 0)
        bad = jnp.zeros((8, 128), F32)
        for par in range(2):
            is_l = (arow < 4 * par) | (arow >= 4 * par + DH)
            hi = jnp.where(is_l, 2.0 ** 60, 2.0 ** 100)
            v = jnp.where(st_ref[par, 0:VROWS, :] <= hi, 0.0, 1.0)
            bad = bad + v[0:8] + v[8:16] + v[16:24]
            is_l8 = (lrow >= 4) if par == 0 else (lrow < 4)
            low = jnp.where(st_ref[par, VROWS:VROWS + 8, :] >= 2.0 ** -30, 0.0, 1.0)
            bad = bad + jnp.where(is_l8, low, 0.0)
        nbad = jnp.sum(bad)

        @pl.when(nbad > 0.0)
        def _():
            def item(t, carry):
                h = lax.shift_right_logical(t, 2)
                q0 = pl.multiple_of(lax.bitwise_and(t, NQ - 1) * BQ, BQ)
                qm = pltpu.bitcast(qh_ref[h, :, pl.ds(q0, BQ)], BF16)

                def chunk(c, st):
                    m, acc = st
                    kl = pltpu.bitcast(
                        kh_ref[h, pl.ds(pl.multiple_of(c * (KC // 2), KC // 2), KC // 2), :], BF16)[:, 0:32]
                    s = lax.dot_general(kl, qm, NN, preferred_element_type=F32)
                    m_new = jnp.maximum(m, jnp.max(s, axis=0, keepdims=True))
                    p = jnp.exp2(s - m_new).astype(BF16)
                    r = lax.dot_general(vt_ref[h, :, pl.ds(pl.multiple_of(c * KC, KC), KC)], p, NN,
                                        preferred_element_type=F32)
                    return m_new, acc * jnp.exp2(m - m_new) + r

                m0 = jnp.full((1, BQ), -jnp.inf, F32)
                _, acc = lax.fori_loop(0, NC, chunk, (m0, jnp.zeros((VROWS, BQ), F32)))
                ot_ref[h, :, pl.ds(q0, BQ)] = acc
                return carry
            lax.fori_loop(0, H * NQ, item, 0)

        for cp in late_copies():
            cp.wait()

    r0 = pl.multiple_of(i * BO, BO)
    xq = x_ref[pl.ds(r0, BO), :]

    hh = jnp.dot(xq, w1_ref[...], preferred_element_type=F32)
    hh = jnp.maximum(hh, 0.0).astype(BF16)
    b = jnp.dot(hh, w2_ref[...], preferred_element_type=F32)

    row8 = lax.broadcasted_iota(jnp.int32, (8, BO), 0)
    blocks = []
    for pair in range(H // 2):
        ae = ot_ref[2 * pair, :, pl.ds(r0, BO)]
        ao = ot_ref[2 * pair + 1, :, pl.ds(r0, BO)]
        ae = ae * (1.0 / ae[20:21, :])
        ao = ao * (1.0 / ao[0:1, :])
        blocks.append(ae[0:16, :])
        blocks.append(jnp.where(row8 < 4, ae[16:24, :], ao[0:8, :]))
        blocks.append(ao[8:24, :])
    o = jnp.concatenate(blocks, axis=0).T.astype(BF16)
    a = jnp.dot(o, wo_ref[...], preferred_element_type=F32)

    gw = gw_ref[...].astype(F32).reshape(1, D)
    z = jnp.sum(xq.astype(F32) * gw, axis=-1, keepdims=True)
    g = jax.nn.sigmoid(z)
    o_ref[...] = (g * a + (1.0 - g) * b).astype(o_ref.dtype)


@jax.jit
def pallas_gated_mix__softmax_full_mha__dense_activation_relu__prompt_kernel(
    A_x: jax.Array,
    A_wqkv: jax.Array,
    A_wo: jax.Array,
    B_x: jax.Array,
    B_w1: jax.Array,
    B_w2: jax.Array,
    gate_w: jax.Array,
):
    del B_x
    anyspec = pl.BlockSpec(memory_space=pl.ANY)
    out = pl.pallas_call(
        _kernel,
        grid=(NO,),
        in_specs=[anyspec] * 6,
        out_specs=pl.BlockSpec((BO, D), lambda i: (i, 0)),
        out_shape=jax.ShapeDtypeStruct((S, D), BF16),
        scratch_shapes=[
            pltpu.VMEM((S, D), BF16),
            pltpu.VMEM((D, 3 * D), BF16),
            pltpu.VMEM((D, D), BF16),
            pltpu.VMEM((D, DFF), BF16),
            pltpu.VMEM((DFF, D), BF16),
            pltpu.VMEM((D,), BF16),
            pltpu.SemaphoreType.DMA((NRA + 7,)),
            pltpu.VMEM((D, D), BF16),
            pltpu.VMEM((H, S // 2, 128), U32),
            pltpu.VMEM((H, VROWS, S), F32),
            pltpu.VMEM((H, 16, S), U32),
            pltpu.VMEM((H, VROWS, S), F32),
            pltpu.VMEM((H, NC * KV, 128), F32),
            pltpu.VMEM((1, NCT // JB, DH, 8, JB * 128), F32),
            pltpu.VMEM((1, NCT // JB, DH, 8, JB * 128), F32),
            pltpu.VMEM((NSLOT, KC, BQ), F32),
            pltpu.VMEM((H, VROWS, S), F32),
            pltpu.VMEM((2, VROWS + 8, 128), F32),
        ] + [pltpu.VMEM((1, DH, KV, 128), F32) for _ in range(NR)],
        compiler_params=pltpu.CompilerParams(
            dimension_semantics=("arbitrary",),
            vmem_limit_bytes=100 * 1024 * 1024),
    )(A_x.reshape(S, D), A_wqkv, A_wo, B_w1, B_w2, gate_w)
    return out.reshape(1, S, D)
```

```python
import math

import jax
import jax.numpy as jnp
from jax import lax
import jax.experimental.pallas as pl
import jax.experimental.pallas.tpu as pltpu

S = 2048
D = 640
H = 32
DH = 20
DFF = 1536

NWIN = 6
VROWS = 24
KC = 128
KV = 16
KM = KC - KV
KO = 2 * KV
GV = KV // 8
NC = S // KC
BQ = 512
NQ = S // BQ
NJ = BQ // 128
NCT = S // 128
NSTEP = NQ * NC
JB = 2

RA = 512
RB = 512
BP = 128
NRA, NRB, NOB = S // RA, S // RB, S // BP

SK = 2
NSLOT = 8
AH = 1
LEAD = 2
NR = 4
PEND = 60
FFN_STEPS = tuple(k for k in range(NSTEP) if (k // NQ) % 4 == 3 and k != 12)
TDS = (5, 15)
TR, TRF, TRX, ER = (3, 6, 10, 13), (5, 9, 13, 15), (1, 4, 7, 10), (2, 5, 8, 11)
PR, PRF = 8, 11

QSCALE = (DH ** -0.5) * math.log2(math.e)

NN = (((1,), (0,)), ((), ()))
NT = (((1,), (1,)), ((), ()))
TN = (((0,), (1,)), ((), ()))
F32 = jnp.float32
BF16 = jnp.bfloat16
U32 = jnp.uint32

SEM_X, SEM_W, SEM_LATE = 0, NRA, NRA + 3
SEM_W1, SEM_W2, SEM_OUT = NRA + 5, NRA + 5 + NRB, NRA + 5 + 2 * NRB
NSEM = SEM_OUT + NOB


def _window(a, w):
    c0 = 120 * w
    g0 = c0 // 128
    g1 = min(c0 + 119, D - 1) // 128
    lo = a[:, g0 * 128:(g0 + 1) * 128]
    if g1 == g0:
        return lo
    lane = lax.broadcasted_iota(jnp.int32, lo.shape, 1)
    return jnp.where(lane >= (c0 % 128), lo, a[:, g1 * 128:(g1 + 1) * 128])


def _part(n, k, nsteps):
    return range((k * n) // nsteps, ((k + 1) * n) // nsteps) if k < nsteps else range(0)


def _recip(l):
    r = pl.reciprocal(l, approx=True)
    r = r * (2.0 - l * r)
    return r * (2.0 - l * r)


def _kernel(x_hbm, wqkv_hbm, wo_hbm, w1_hbm, w2_hbm, gw_hbm, o_hbm,
            x_ref, wqkv_ref, wo_ref, w1_ref, w2_ref, gw_ref, sems,
            kh_ref, vt_ref, qh_ref, qt_ref, koff_ref, qba_ref, qbb_ref, pb_ref, ot_ref, st_ref, wqt_ref,
            ha_ref, h1_ref, b_ref, xp_ref, w1p_ref, w2p_ref, ob_ref, *kb_refs):
    i = pl.program_id(0)
    qb_refs = (qba_ref, qbb_ref)

    def x_copy(c):
        r = pl.multiple_of(c * RA, RA)
        return pltpu.make_async_copy(x_hbm.at[pl.ds(r, RA), :], x_ref.at[pl.ds(r, RA), :], sems.at[SEM_X + c])

    def w_copy(j):
        return pltpu.make_async_copy(wqkv_hbm.at[:, pl.ds(j * D, D)], wqkv_ref.at[:, pl.ds(j * D, D)],
                                     sems.at[SEM_W + j])

    def late_copies():
        return [pltpu.make_async_copy(wo_hbm, wo_ref, sems.at[SEM_LATE]),
                pltpu.make_async_copy(gw_hbm, gw_ref, sems.at[SEM_LATE + 1])]

    def ffn_copies(c):
        n1, n2 = D // NRB, DFF // NRB
        r1, r2 = pl.multiple_of(c * n1, 16), pl.multiple_of(c * n2, 16)
        return [pltpu.make_async_copy(w1_hbm.at[pl.ds(r1, n1), :], w1_ref.at[pl.ds(r1, n1), :],
                                      sems.at[SEM_W1 + c]),
                pltpu.make_async_copy(w2_hbm.at[pl.ds(r2, n2), :], w2_ref.at[pl.ds(r2, n2), :],
                                      sems.at[SEM_W2 + c])]

    @pl.when(i == 0)
    def _():
        w_copy(0).start()
        x_copy(0).start()
        for k in range(NSTEP - SK, NSTEP):
            pb_ref[k % NSLOT] = jnp.ones((KC, BQ), F32)
            ot_ref[1, :, (k % NQ) * BQ:(k % NQ + 1) * BQ] = jnp.zeros((VROWS, BQ), F32)
        st_ref[:, 0:VROWS, :] = jnp.zeros((2, VROWS, 128), F32)
        st_ref[:, VROWS:VROWS + 8, :] = jnp.ones((2, 8, 128), F32)
        w_copy(0).wait()
        for c in range(1, NRA):
            x_copy(c).start()
        w_copy(1).start()
        w_copy(2).start()
        for c in range(NRB):
            for cp in ffn_copies(c):
                cp.start()
        for cp in late_copies():
            cp.start()
        wqt_ref[...] = wqkv_ref[:, 0:D].T

        def proj_q(c, carry):
            r0 = pl.multiple_of(c * RA, RA)
            x_copy(c).wait()
            xc = x_ref[pl.ds(r0, RA), :]
            xp_ref[pl.ds(pl.multiple_of(c * (RA // 2), RA // 2), RA // 2), :] = pltpu.bitcast(xc, U32)
            qt = lax.dot_general(wqt_ref[...], xc, NT, preferred_element_type=F32) * QSCALE
            qt = qt.astype(BF16).astype(F32)
            zpad = jnp.zeros((32 - DH, RA), F32)
            for h in range(H):
                rows = qt[DH * h:DH * h + DH, :]
                qh_ref[h, :, pl.ds(r0, RA)] = pltpu.bitcast(
                    jnp.concatenate([rows, zpad], axis=0).astype(BF16), U32)
                qt_ref[h, 0:DH, pl.ds(r0, RA)] = rows
                if h == 0:
                    nb = RA // (JB * 128)
                    for b in range(nb):
                        for d in range(DH):
                            qba_ref[0, c * nb + b, d] = jnp.broadcast_to(
                                rows[d:d + 1, b * JB * 128:(b + 1) * JB * 128], (8, JB * 128))
            return carry
        lax.fori_loop(0, NRA, proj_q, 0)
        w_copy(1).wait()
        w_copy(2).wait()

        def proj_kv(c, carry):
            r0 = pl.multiple_of(c * RB, RB)
            for cp in ffn_copies(c):
                cp.wait()
            xc = x_ref[pl.ds(r0, RB), :]
            k = jnp.dot(xc, wqkv_ref[:, D:2 * D], preferred_element_type=F32).astype(BF16).astype(F32)
            r0h = pl.multiple_of(c * (RB // 2), RB // 2)
            n1, n2 = D // NRB, DFF // NRB
            p1 = pltpu.bitcast(w1_ref[pl.ds(pl.multiple_of(c * n1, 16), n1), :], U32)
            p2 = pltpu.bitcast(w2_ref[pl.ds(pl.multiple_of(c * n2, 16), n2), :], U32)
            kbits = pltpu.bitcast(k[:, D - 128:D], U32)
            p1 = jnp.where(lax.broadcasted_iota(jnp.int32, p1.shape, 1) < (i - 1),
                           jnp.concatenate([kbits[0:n1 // 2]] * (DFF // 128), axis=1), p1)
            p2 = jnp.where(lax.broadcasted_iota(jnp.int32, p2.shape, 1) < (i - 1),
                           jnp.concatenate([kbits[RB - n2 // 2:RB]] * (D // 128), axis=1), p2)
            w1p_ref[pl.ds(pl.multiple_of(c * (n1 // 2), 8), n1 // 2), :] = p1
            w2p_ref[pl.ds(pl.multiple_of(c * (n2 // 2), 8), n2 // 2), :] = p2
            no = RB // KC * KO
            for w in range(NWIN):
                kwin = _window(k, w)
                kpk = pltpu.bitcast(kwin.astype(BF16), U32)
                ko = jnp.concatenate([kwin[b * KC + KC - KO:(b + 1) * KC, :] for b in range(RB // KC)], axis=0)
                for h in range(6 * w, min(6 * w + 6, H)):
                    off = (DH * h) % 128
                    kh_ref[h, pl.ds(r0h, RB // 2), :] = pltpu.roll(kpk, 128 - off, 1) if off else kpk
                    koff_ref[h, pl.ds(pl.multiple_of(c * no, no), no), :] = (
                        pltpu.roll(ko, 128 - off, 1) if off else ko)
            vt = lax.dot_general(wqkv_ref[:, 2 * D:3 * D], xc, TN, preferred_element_type=F32)
            row = lax.broadcasted_iota(jnp.int32, (VROWS, RB), 0)
            for h in range(H):
                st = (DH * h) // 8 * 8
                off = DH * h - st
                blk = vt[st:st + VROWS, :]
                vt_ref[h, :, pl.ds(r0, RB)] = jnp.where((row >= off) & (row < off + DH), blk, 1.0)
            return carry
        lax.fori_loop(0, NRB, proj_kv, 0)

        fmask = lax.broadcasted_iota(jnp.int32, (8, 128), 1) < (i - 1)
        fmask3 = jnp.concatenate([jnp.concatenate([fmask] * GV, axis=0)] * JB, axis=1)

        def tie_rows(s, r, j0, w):
            r = min(r, s.shape[0] // 8 - 1)
            if s.shape[1] >= (j0 + w) * 128:
                return s[8 * r:8 * r + 8, j0 * 128:(j0 + w) * 128]
            return jnp.concatenate([s[8 * r:8 * r + 8, 0:128]] * w, axis=1)

        def prep_qb(hh, par, k, tie):
            for e in _part(DH * NCT, k, PEND):
                ct, d = e // DH, e % DH
                v = jnp.broadcast_to(qt_ref[hh, d:d + 1, ct * 128:(ct + 1) * 128], (8, 128))
                if tie is not None:
                    v = jnp.where(fmask, tie, v)
                qb_refs[par][0, ct // JB, d, :, (ct % JB) * 128:(ct % JB + 1) * 128] = v

        def prep_kb(hh, c, k, nsteps, tie):
            n = KO if c % 4 == 3 else KV
            kv = koff_ref[hh, (c + 1) * KO - n:(c + 1) * KO, :]
            if tie is not None:
                kv = jnp.where(jnp.concatenate([fmask] * (n // 8), axis=0),
                               jnp.concatenate([tie] * (n // 8), axis=0), kv)
            for d in _part(DH, k, nsteps):
                kb_refs[c % NR][0, :, d] = jnp.broadcast_to(kv[:, d:d + 1], (n, 128)).reshape(n // KV, KV, 128)

        def vpu_scores(par, k, zbase, last, tr, band=0):
            c, qb = k // NQ, k % NQ
            nb = 2 if c % 4 == 3 else 1
            for j0 in range(0, NJ, JB):
                zk = 0 if zbase is None else i * (NSTEP + 1 + (zbase * 2 + band) * NJ + j0)
                kb = kb_refs[c % NR][zk, nb - 1 - band]
                qv = qb_refs[par][zk, (qb * NJ + j0) // JB]
                terms = jnp.concatenate([kb] * JB, axis=2) * jnp.concatenate([qv] * GV, axis=1)
                if last is not None:
                    segs, d0 = [], 0
                    for n, d in enumerate(TDS):
                        tie = tie_rows(last, tr[(j0 // JB) * len(TDS) + n], j0, JB)
                        segs.append(terms[d0:d])
                        segs.append(jnp.where(fmask3[None], jnp.concatenate([tie] * GV, axis=0)[None],
                                              terms[d:d + 1]))
                        d0 = d + 1
                    segs.append(terms[d0:DH])
                    terms = jnp.concatenate(segs, axis=0)
                lo = KM - KV * band
                pb_ref[k % NSLOT, lo:lo + KV, j0 * 128:(j0 + JB) * 128] = jnp.exp2(jnp.sum(terms, axis=0))

        def ffn_slice(u, par, n):
            if par == 0:
                ng, kt = n // 5, n % 5
                f = jnp.dot(
                    pltpu.bitcast(xp_ref[pl.ds(pl.multiple_of(u * 64, 64), 64), kt * 128:(kt + 1) * 128], BF16),
                    pltpu.bitcast(w1p_ref[kt * 64:(kt + 1) * 64, ng * 512:(ng + 1) * 512], BF16),
                    preferred_element_type=F32)
                t = f if kt == 0 else f + ha_ref[...]
                if kt < 4:
                    ha_ref[...] = t
                else:
                    h1_ref[:, ng * 512:(ng + 1) * 512] = pltpu.bitcast(jnp.maximum(t, 0.0).astype(BF16), U32)
            else:
                nt, kg = n // 3, n % 3
                rr = pl.multiple_of(u * 128, 128)
                f = jnp.dot(
                    pltpu.bitcast(h1_ref[:, kg * 512:(kg + 1) * 512], BF16),
                    pltpu.bitcast(w2p_ref[kg * 256:(kg + 1) * 256, nt * 128:(nt + 1) * 128], BF16),
                    preferred_element_type=F32)
                t = f if kg == 0 else f + b_ref[pl.ds(rr, 128), nt * 128:(nt + 1) * 128]
                b_ref[pl.ds(rr, 128), nt * 128:(nt + 1) * 128] = t
            return f

        def do_pv(h, par, kk):
            c, qb = kk // NQ, kk % NQ
            p = pb_ref[kk % NSLOT].astype(BF16)
            r = lax.dot_general(vt_ref[h, :, c * KC:(c + 1) * KC], p, NN, preferred_element_type=F32)
            if c > 0:
                r = r + ot_ref[h, :, qb * BQ:(qb + 1) * BQ]
            ot_ref[h, :, qb * BQ:(qb + 1) * BQ] = r
            if c == NC - 1:
                a = jnp.abs(r)
                mx = jnp.maximum(jnp.maximum(a[:, 0:128], a[:, 128:256]),
                                 jnp.maximum(a[:, 256:384], a[:, 384:512]))
                st_ref[par, 0:VROWS, :] = jnp.maximum(st_ref[par, 0:VROWS, :], mx)
                lr = r[16:24, :] if par == 0 else r[0:8, :]
                mn = jnp.minimum(jnp.minimum(lr[:, 0:128], lr[:, 128:256]),
                                 jnp.minimum(lr[:, 256:384], lr[:, 384:512]))
                st_ref[par, VROWS:VROWS + 8, :] = jnp.minimum(st_ref[par, VROWS:VROWS + 8, :], mn)

        for c in range(LEAD):
            prep_kb(0, c, 0, 1, None)
        for k in range(AH + 1):
            vpu_scores(0, k, None, None, TR)

        def head_pair(u, carry):
            last, ltr, lpr = None, TR, PR
            for par in range(2):
                h = 2 * u + par
                hn = h + 1 if par == 0 else jnp.minimum(h + 1, H - 1)
                hp = h - 1 if par == 1 else jnp.maximum(h - 1, 1)
                for k in range(NSTEP):
                    c, qb = k // NQ, k % NQ
                    ff = k in FFN_STEPS
                    km = KM - KV if ff else KM
                    kl = pltpu.bitcast(kh_ref[h, c * KC // 2:(c * KC + km) // 2, :], BF16)[:, 0:32]
                    qm = pltpu.bitcast(qh_ref[h + i * (k + 1), :, qb * BQ:(qb + 1) * BQ], BF16)
                    s = lax.dot_general(kl, qm, NN, preferred_element_type=F32)
                    pb_ref[k % NSLOT, 0:km, :] = jnp.exp2(s)
                    if last is None:
                        pass
                    elif k + AH < NSTEP:
                        vpu_scores(par, k + AH, k, last, ltr)
                    else:
                        vpu_scores(1 - par, k + AH - NSTEP, k, last, ltr)
                    tie = None if last is None else last[8 * lpr:8 * lpr + 8, 0:128]
                    prep_qb(hn, 1 - par, k, tie)
                    if c + LEAD < NC:
                        prep_kb(h, c + LEAD, qb, NQ, tie)
                    else:
                        prep_kb(hn, c + LEAD - NC, qb, NQ, tie)
                    if ff:
                        f = ffn_slice(u, par, FFN_STEPS.index(k))
                    if k >= SK:
                        do_pv(h, par, k - SK)
                    else:
                        do_pv(hp, 1 - par, NSTEP + k - SK)
                    last, ltr, lpr = s, TR, PR
                    if ff:
                        vpu_scores(par, k, k, s, TRX, band=1)
                        last, ltr, lpr = f, TRF, PRF
            vpu_scores(0, AH, NSTEP * 20, last, ER)
            return carry

        lax.fori_loop(0, H // 2, head_pair, 0)
        for k in range(SK):
            do_pv(H - 1, 1, NSTEP + k - SK)

        arow = lax.broadcasted_iota(jnp.int32, (VROWS, 128), 0)
        lrow = lax.broadcasted_iota(jnp.int32, (8, 128), 0)
        bad = jnp.zeros((8, 128), F32)
        for par in range(2):
            is_l = (arow < 4 * par) | (arow >= 4 * par + DH)
            hi = jnp.where(is_l, 2.0 ** 60, 2.0 ** 100)
            v = jnp.where(st_ref[par, 0:VROWS, :] <= hi, 0.0, 1.0)
            bad = bad + v[0:8] + v[8:16] + v[16:24]
            is_l8 = (lrow >= 4) if par == 0 else (lrow < 4)
            low = jnp.where(st_ref[par, VROWS:VROWS + 8, :] >= 2.0 ** -30, 0.0, 1.0)
            bad = bad + jnp.where(is_l8, low, 0.0)
        nbad = jnp.sum(bad)

        @pl.when(nbad > 0.0)
        def _():
            def item(t, carry):
                h = lax.shift_right_logical(t, 2)
                q0 = pl.multiple_of(lax.bitwise_and(t, NQ - 1) * BQ, BQ)
                qm = pltpu.bitcast(qh_ref[h, :, pl.ds(q0, BQ)], BF16)

                def chunk(c, st):
                    m, acc = st
                    kl = pltpu.bitcast(
                        kh_ref[h, pl.ds(pl.multiple_of(c * (KC // 2), KC // 2), KC // 2), :], BF16)[:, 0:32]
                    s = lax.dot_general(kl, qm, NN, preferred_element_type=F32)
                    m_new = jnp.maximum(m, jnp.max(s, axis=0, keepdims=True))
                    p = jnp.exp2(s - m_new).astype(BF16)
                    r = lax.dot_general(vt_ref[h, :, pl.ds(pl.multiple_of(c * KC, KC), KC)], p, NN,
                                        preferred_element_type=F32)
                    return m_new, acc * jnp.exp2(m - m_new) + r

                m0 = jnp.full((1, BQ), -jnp.inf, F32)
                _, acc = lax.fori_loop(0, NC, chunk, (m0, jnp.zeros((VROWS, BQ), F32)))
                ot_ref[h, :, pl.ds(q0, BQ)] = acc
                return carry
            lax.fori_loop(0, H * NQ, item, 0)

        for cp in late_copies():
            cp.wait()

    @pl.when(i == 1)
    def _():
        def out_copy(j):
            return pltpu.make_async_copy(ob_ref.at[pl.ds(j * BP, BP), :], o_hbm.at[pl.ds(j * BP, BP), :],
                                         sems.at[SEM_OUT + j])

        row8 = lax.broadcasted_iota(jnp.int32, (8, BP), 0)
        for j in range(NOB):
            rows = slice(j * BP, (j + 1) * BP)
            blocks = []
            for pair in range(H // 2):
                ae = ot_ref[2 * pair, :, rows]
                ao = ot_ref[2 * pair + 1, :, rows]
                ae = ae * _recip(ae[20:21, :])
                ao = ao * _recip(ao[0:1, :])
                blocks.append(ae[0:16, :])
                blocks.append(jnp.where(row8 < 4, ae[16:24, :], ao[0:8, :]))
                blocks.append(ao[8:24, :])
            o = jnp.concatenate(blocks, axis=0).T.astype(BF16)
            a = jnp.dot(o, wo_ref[...], preferred_element_type=F32)
            gw = gw_ref[...].astype(F32).reshape(1, D)
            z = jnp.sum(x_ref[rows, :].astype(F32) * gw, axis=-1, keepdims=True)
            g = jax.nn.sigmoid(z)
            ob_ref[rows, :] = (g * a + (1.0 - g) * b_ref[rows, :]).astype(BF16)
            out_copy(j).start()
        for j in range(NOB):
            out_copy(j).wait()


@jax.jit
def pallas_gated_mix__softmax_full_mha__dense_activation_relu__prompt_kernel(
    A_x: jax.Array,
    A_wqkv: jax.Array,
    A_wo: jax.Array,
    B_x: jax.Array,
    B_w1: jax.Array,
    B_w2: jax.Array,
    gate_w: jax.Array,
):
    del B_x
    anyspec = pl.BlockSpec(memory_space=pl.ANY)
    out = pl.pallas_call(
        _kernel,
        grid=(2,),
        in_specs=[anyspec] * 6,
        out_specs=anyspec,
        out_shape=jax.ShapeDtypeStruct((S, D), BF16),
        scratch_shapes=[
            pltpu.VMEM((S, D), BF16),
            pltpu.VMEM((D, 3 * D), BF16),
            pltpu.VMEM((D, D), BF16),
            pltpu.VMEM((D, DFF), BF16),
            pltpu.VMEM((DFF, D), BF16),
            pltpu.VMEM((D,), BF16),
            pltpu.SemaphoreType.DMA((NSEM,)),
            pltpu.VMEM((H, S // 2, 128), U32),
            pltpu.VMEM((H, VROWS, S), F32),
            pltpu.VMEM((H, 16, S), U32),
            pltpu.VMEM((H, VROWS, S), F32),
            pltpu.VMEM((H, NC * KO, 128), F32),
            pltpu.VMEM((1, NCT // JB, DH, 8, JB * 128), F32),
            pltpu.VMEM((1, NCT // JB, DH, 8, JB * 128), F32),
            pltpu.VMEM((NSLOT, KC, BQ), F32),
            pltpu.VMEM((H, VROWS, S), F32),
            pltpu.VMEM((2, VROWS + 8, 128), F32),
            pltpu.VMEM((D, D), BF16),
            pltpu.VMEM((128, 512), F32),
            pltpu.VMEM((64, DFF), U32),
            pltpu.VMEM((S, D), F32),
            pltpu.VMEM((S // 2, D), U32),
            pltpu.VMEM((D // 2, DFF), U32),
            pltpu.VMEM((DFF // 2, D), U32),
            pltpu.VMEM((S, D), BF16),
        ] + [pltpu.VMEM((1, 2 if r == 3 else 1, DH, KV, 128), F32) for r in range(NR)],
        compiler_params=pltpu.CompilerParams(
            dimension_semantics=("arbitrary",),
            vmem_limit_bytes=100 * 1024 * 1024),
    )(A_x.reshape(S, D), A_wqkv, A_wo, B_w1, B_w2, gate_w)
    return out.reshape(1, S, D)
```

```python
import math

import jax
import jax.numpy as jnp
from jax import lax
import jax.experimental.pallas as pl
import jax.experimental.pallas.tpu as pltpu

S = 2048
D = 640
H = 32
DH = 20
DFF = 1536

NWIN = 6
VROWS = 24
KC = 128
KV = 16
KM = KC - KV
KO = 2 * KV
KG = 3 * KV + KO
GV = KV // 8
NC = S // KC
BQ = 512
NQ = S // BQ
NJ = BQ // 128
NCT = S // 128
NSTEP = NQ * NC
JB = 2

RA = 512
RB = 1024
BP = 128
NRA, NRB, NOB = S // RA, S // RB, S // BP

SK = 2
NSLOT = 8
AH = 1
LEAD = 2
NR = 4
PEND = 60
FFN_STEPS = tuple(k for k in range(NSTEP) if (k // NQ) % 4 == 3 and k != 12)
TDS = (5, 15)
TR, TRF, TRX, ER = (3, 6, 10, 13), (5, 9, 13, 15), (1, 4, 7, 10), (2, 5, 8, 11)
PR, PRF = 8, 11

QSCALE = (DH ** -0.5) * math.log2(math.e)

NN = (((1,), (0,)), ((), ()))
NT = (((1,), (1,)), ((), ()))
TN = (((0,), (1,)), ((), ()))
F32 = jnp.float32
BF16 = jnp.bfloat16
U32 = jnp.uint32

SEM_X, SEM_W, SEM_LATE = 0, NRA, NRA + 3
SEM_W1, SEM_W2, SEM_OUT = NRA + 5, NRA + 5 + NRB, NRA + 5 + 2 * NRB
NSEM = SEM_OUT + NOB


def _window(a, w):
    c0 = 120 * w
    g0 = c0 // 128
    g1 = min(c0 + 119, D - 1) // 128
    lo = a[:, g0 * 128:(g0 + 1) * 128]
    if g1 == g0:
        return lo
    lane = lax.broadcasted_iota(jnp.int32, lo.shape, 1)
    return jnp.where(lane >= (c0 % 128), lo, a[:, g1 * 128:(g1 + 1) * 128])


def _part(n, k, nsteps):
    return range((k * n) // nsteps, ((k + 1) * n) // nsteps) if k < nsteps else range(0)


def _recip(l):
    r = pl.reciprocal(l, approx=True)
    return r * (2.0 - l * r)


def _kernel(x_hbm, wqkv_hbm, wo_hbm, w1_hbm, w2_hbm, gw_hbm, o_hbm,
            x_ref, wqkv_ref, wo_ref, w1_ref, w2_ref, gw_ref, sems,
            kh_ref, vt_ref, qh_ref, qt_ref, koff_ref, qba_ref, qbb_ref, pb_ref, ot_ref, st_ref, wqt_ref,
            ha_ref, h1_ref, b_ref, xp_ref, w1p_ref, w2p_ref, ob_ref, *kb_refs):
    i = pl.program_id(0)
    qb_refs = (qba_ref, qbb_ref)

    def x_copy(c):
        r = pl.multiple_of(c * RA, RA)
        return pltpu.make_async_copy(x_hbm.at[pl.ds(r, RA), :], x_ref.at[pl.ds(r, RA), :], sems.at[SEM_X + c])

    def w_copy(j):
        return pltpu.make_async_copy(wqkv_hbm.at[:, pl.ds(j * D, D)], wqkv_ref.at[:, pl.ds(j * D, D)],
                                     sems.at[SEM_W + j])

    def late_copies():
        return [pltpu.make_async_copy(wo_hbm, wo_ref, sems.at[SEM_LATE]),
                pltpu.make_async_copy(gw_hbm, gw_ref, sems.at[SEM_LATE + 1])]

    def ffn_copies(c):
        n1, n2 = D // NRB, DFF // NRB
        r1, r2 = pl.multiple_of(c * n1, 16), pl.multiple_of(c * n2, 16)
        return [pltpu.make_async_copy(w1_hbm.at[pl.ds(r1, n1), :], w1_ref.at[pl.ds(r1, n1), :],
                                      sems.at[SEM_W1 + c]),
                pltpu.make_async_copy(w2_hbm.at[pl.ds(r2, n2), :], w2_ref.at[pl.ds(r2, n2), :],
                                      sems.at[SEM_W2 + c])]

    @pl.when(i == 0)
    def _():
        w_copy(0).start()
        x_copy(0).start()
        for k in range(NSTEP - SK, NSTEP):
            pb_ref[k % NSLOT] = jnp.ones((KC, BQ), F32)
            ot_ref[1, :, (k % NQ) * BQ:(k % NQ + 1) * BQ] = jnp.zeros((VROWS, BQ), F32)
        st_ref[:, 0:VROWS, :] = jnp.zeros((2, VROWS, 128), F32)
        st_ref[:, VROWS:VROWS + 8, :] = jnp.ones((2, 8, 128), F32)
        w_copy(0).wait()
        for c in range(1, NRA):
            x_copy(c).start()
        w_copy(1).start()
        w_copy(2).start()
        for c in range(NRB):
            for cp in ffn_copies(c):
                cp.start()
        for cp in late_copies():
            cp.start()
        wqt_ref[...] = wqkv_ref[:, 0:D].T

        def proj_q(c, carry):
            r0 = pl.multiple_of(c * RA, RA)
            x_copy(c).wait()
            xc = x_ref[pl.ds(r0, RA), :]
            xp_ref[pl.ds(pl.multiple_of(c * (RA // 2), RA // 2), RA // 2), :] = pltpu.bitcast(xc, U32)
            qt = lax.dot_general(wqt_ref[...], xc, NT, preferred_element_type=F32) * QSCALE
            qt = qt.astype(BF16).astype(F32)
            zpad = jnp.zeros((32 - DH, RA), F32)
            for h in range(H):
                rows = qt[DH * h:DH * h + DH, :]
                qh_ref[h, :, pl.ds(r0, RA)] = pltpu.bitcast(
                    jnp.concatenate([rows, zpad], axis=0).astype(BF16), U32)
                qt_ref[h, 0:DH, pl.ds(r0, RA)] = rows
                if h == 0:
                    nb = RA // (JB * 128)
                    for b in range(nb):
                        for d in range(DH):
                            qba_ref[0, c * nb + b, d] = jnp.broadcast_to(
                                rows[d:d + 1, b * JB * 128:(b + 1) * JB * 128], (8, JB * 128))
            return carry
        lax.fori_loop(0, NRA, proj_q, 0)
        w_copy(1).wait()
        w_copy(2).wait()

        def proj_kv(c, carry):
            r0 = pl.multiple_of(c * RB, RB)
            for cp in ffn_copies(c):
                cp.wait()
            xc = x_ref[pl.ds(r0, RB), :]
            k = jnp.dot(xc, wqkv_ref[:, D:2 * D], preferred_element_type=F32).astype(BF16).astype(F32)
            r0h = pl.multiple_of(c * (RB // 2), RB // 2)
            no = RB // (4 * KC) * KG
            for w in range(NWIN):
                kwin = _window(k, w)
                kpk = pltpu.bitcast(kwin.astype(BF16), U32)
                ko = jnp.concatenate([kwin[(b + 1) * KC - (KO if b % 4 == 3 else KV):(b + 1) * KC, :]
                                      for b in range(RB // KC)], axis=0)
                for h in range(6 * w, min(6 * w + 6, H)):
                    off = (DH * h) % 128
                    kh_ref[h, pl.ds(r0h, RB // 2), :] = pltpu.roll(kpk, 128 - off, 1) if off else kpk
                    koff_ref[h, pl.ds(pl.multiple_of(c * no, 8), no), :] = (
                        pltpu.roll(ko, 128 - off, 1) if off else ko)
            vt = lax.dot_general(wqkv_ref[:, 2 * D:3 * D], xc, TN, preferred_element_type=F32)
            n1, n2 = D // NRB, DFF // NRB
            p1 = pltpu.bitcast(w1_ref[pl.ds(pl.multiple_of(c * n1, 16), n1), :], U32)
            p2 = pltpu.bitcast(w2_ref[pl.ds(pl.multiple_of(c * n2, 16), n2), :], U32)
            kbits = pltpu.bitcast(vt[:, RB - 128:RB], U32)
            p1 = jnp.where(lax.broadcasted_iota(jnp.int32, p1.shape, 1) < (i - 1),
                           jnp.concatenate([kbits[0:n1 // 2]] * (DFF // 128), axis=1), p1)
            p2 = jnp.where(lax.broadcasted_iota(jnp.int32, p2.shape, 1) < (i - 1),
                           jnp.concatenate([kbits[512 - n2 // 2:512]] * (D // 128), axis=1), p2)
            w1p_ref[pl.ds(pl.multiple_of(c * (n1 // 2), 8), n1 // 2), :] = p1
            w2p_ref[pl.ds(pl.multiple_of(c * (n2 // 2), 8), n2 // 2), :] = p2
            row = lax.broadcasted_iota(jnp.int32, (VROWS, RB), 0)
            for h in range(H):
                st = (DH * h) // 8 * 8
                off = DH * h - st
                blk = vt[st:st + VROWS, :]
                vt_ref[h, :, pl.ds(r0, RB)] = jnp.where((row >= off) & (row < off + DH), blk, 1.0)
            return carry
        lax.fori_loop(0, NRB, proj_kv, 0)

        fmask = lax.broadcasted_iota(jnp.int32, (8, 128), 1) < (i - 1)
        fmask3 = jnp.concatenate([jnp.concatenate([fmask] * GV, axis=0)] * JB, axis=1)

        def tie_rows(s, r, j0, w):
            r = min(r, s.shape[0] // 8 - 1)
            if s.shape[1] >= (j0 + w) * 128:
                return s[8 * r:8 * r + 8, j0 * 128:(j0 + w) * 128]
            return jnp.concatenate([s[8 * r:8 * r + 8, 0:128]] * w, axis=1)

        def prep_qb(hh, par, k, tie):
            for e in _part(DH * NCT, k, PEND):
                ct, d = e // DH, e % DH
                v = jnp.broadcast_to(qt_ref[hh, d:d + 1, ct * 128:(ct + 1) * 128], (8, 128))
                if tie is not None:
                    v = jnp.where(fmask, tie, v)
                qb_refs[par][0, ct // JB, d, :, (ct % JB) * 128:(ct % JB + 1) * 128] = v

        def prep_kb(hh, c, k, nsteps, tie):
            n = KO if c % 4 == 3 else KV
            k0 = (c // 4) * KG + (c % 4) * KV
            kv = koff_ref[hh, k0:k0 + n, :]
            if tie is not None:
                kv = jnp.where(jnp.concatenate([fmask] * (n // 8), axis=0),
                               jnp.concatenate([tie] * (n // 8), axis=0), kv)
            for d in _part(DH, k, nsteps):
                kb_refs[c % NR][0, :, d] = jnp.broadcast_to(kv[:, d:d + 1], (n, 128)).reshape(n // KV, KV, 128)

        def vpu_scores(par, k, zbase, last, tr, band=0):
            c, qb = k // NQ, k % NQ
            nb = 2 if c % 4 == 3 else 1
            for j0 in range(0, NJ, JB):
                zk = 0 if zbase is None else i * (NSTEP + 1 + (zbase * 2 + band) * NJ + j0)
                kb = kb_refs[c % NR][zk, nb - 1 - band]
                qv = qb_refs[par][zk, (qb * NJ + j0) // JB]
                terms = jnp.concatenate([kb] * JB, axis=2) * jnp.concatenate([qv] * GV, axis=1)
                if last is not None:
                    segs, d0 = [], 0
                    for n, d in enumerate(TDS):
                        tie = tie_rows(last, tr[(j0 // JB) * len(TDS) + n], j0, JB)
                        segs.append(terms[d0:d])
                        segs.append(jnp.where(fmask3[None], jnp.concatenate([tie] * GV, axis=0)[None],
                                              terms[d:d + 1]))
                        d0 = d + 1
                    segs.append(terms[d0:DH])
                    terms = jnp.concatenate(segs, axis=0)
                lo = KM - KV * band
                pb_ref[k % NSLOT, lo:lo + KV, j0 * 128:(j0 + JB) * 128] = jnp.exp2(jnp.sum(terms, axis=0))

        def ffn_slice(u, par, n):
            if par == 0:
                ng, kt = n // 5, n % 5
                f = jnp.dot(
                    pltpu.bitcast(xp_ref[pl.ds(pl.multiple_of(u * 64, 64), 64), kt * 128:(kt + 1) * 128], BF16),
                    pltpu.bitcast(w1p_ref[kt * 64:(kt + 1) * 64, ng * 512:(ng + 1) * 512], BF16),
                    preferred_element_type=F32)
                t = f if kt == 0 else f + ha_ref[...]
                if kt < 4:
                    ha_ref[...] = t
                else:
                    h1_ref[:, ng * 512:(ng + 1) * 512] = pltpu.bitcast(jnp.maximum(t, 0.0).astype(BF16), U32)
            else:
                nt, kg = n // 3, n % 3
                rr = pl.multiple_of(u * 128, 128)
                f = jnp.dot(
                    pltpu.bitcast(h1_ref[:, kg * 512:(kg + 1) * 512], BF16),
                    pltpu.bitcast(w2p_ref[kg * 256:(kg + 1) * 256, nt * 128:(nt + 1) * 128], BF16),
                    preferred_element_type=F32)
                t = f if kg == 0 else f + b_ref[pl.ds(rr, 128), nt * 128:(nt + 1) * 128]
                b_ref[pl.ds(rr, 128), nt * 128:(nt + 1) * 128] = t
            return f

        def do_pv(h, par, kk):
            c, qb = kk // NQ, kk % NQ
            p = pb_ref[kk % NSLOT].astype(BF16)
            r = lax.dot_general(vt_ref[h, :, c * KC:(c + 1) * KC], p, NN, preferred_element_type=F32)
            if c > 0:
                r = r + ot_ref[h, :, qb * BQ:(qb + 1) * BQ]
            ot_ref[h, :, qb * BQ:(qb + 1) * BQ] = r
            if c == NC - 1:
                a = jnp.abs(r)
                mx = jnp.maximum(jnp.maximum(a[:, 0:128], a[:, 128:256]),
                                 jnp.maximum(a[:, 256:384], a[:, 384:512]))
                st_ref[par, 0:VROWS, :] = jnp.maximum(st_ref[par, 0:VROWS, :], mx)
                lr = r[16:24, :] if par == 0 else r[0:8, :]
                mn = jnp.minimum(jnp.minimum(lr[:, 0:128], lr[:, 128:256]),
                                 jnp.minimum(lr[:, 256:384], lr[:, 384:512]))
                st_ref[par, VROWS:VROWS + 8, :] = jnp.minimum(st_ref[par, VROWS:VROWS + 8, :], mn)

        for c in range(LEAD):
            prep_kb(0, c, 0, 1, None)
        for k in range(AH + 1):
            vpu_scores(0, k, None, None, TR)

        def head_pair(u, carry):
            last, ltr, lpr = None, TR, PR
            for par in range(2):
                h = 2 * u + par
                hn = h + 1 if par == 0 else jnp.minimum(h + 1, H - 1)
                hp = h - 1 if par == 1 else jnp.maximum(h - 1, 1)
                for k in range(NSTEP):
                    c, qb = k // NQ, k % NQ
                    ff = k in FFN_STEPS
                    km = KM - KV if ff else KM
                    kl = pltpu.bitcast(kh_ref[h, c * KC // 2:(c * KC + km) // 2, :], BF16)[:, 0:32]
                    qm = pltpu.bitcast(qh_ref[h + i * (k + 1), :, qb * BQ:(qb + 1) * BQ], BF16)
                    s = lax.dot_general(kl, qm, NN, preferred_element_type=F32)
                    pb_ref[k % NSLOT, 0:km, :] = jnp.exp2(s)
                    if last is None:
                        pass
                    elif k + AH < NSTEP:
                        vpu_scores(par, k + AH, k, last, ltr)
                    else:
                        vpu_scores(1 - par, k + AH - NSTEP, k, last, ltr)
                    tie = None if last is None else last[8 * lpr:8 * lpr + 8, 0:128]
                    prep_qb(hn, 1 - par, k, tie)
                    if c + LEAD < NC:
                        prep_kb(h, c + LEAD, qb, NQ, tie)
                    else:
                        prep_kb(hn, c + LEAD - NC, qb, NQ, tie)
                    if ff:
                        f = ffn_slice(u, par, FFN_STEPS.index(k))
                    if k >= SK:
                        do_pv(h, par, k - SK)
                    else:
                        do_pv(hp, 1 - par, NSTEP + k - SK)
                    last, ltr, lpr = s, TR, PR
                    if ff:
                        vpu_scores(par, k, k, s, TRX, band=1)
                        last, ltr, lpr = f, TRF, PRF
            vpu_scores(0, AH, NSTEP * 20, last, ER)
            return carry

        lax.fori_loop(0, H // 2, head_pair, 0)
        for k in range(SK):
            do_pv(H - 1, 1, NSTEP + k - SK)

        arow = lax.broadcasted_iota(jnp.int32, (VROWS, 128), 0)
        lrow = lax.broadcasted_iota(jnp.int32, (8, 128), 0)
        bad = jnp.zeros((8, 128), F32)
        for par in range(2):
            is_l = (arow < 4 * par) | (arow >= 4 * par + DH)
            hi = jnp.where(is_l, 2.0 ** 60, 2.0 ** 100)
            v = jnp.where(st_ref[par, 0:VROWS, :] <= hi, 0.0, 1.0)
            bad = bad + v[0:8] + v[8:16] + v[16:24]
            is_l8 = (lrow >= 4) if par == 0 else (lrow < 4)
            low = jnp.where(st_ref[par, VROWS:VROWS + 8, :] >= 2.0 ** -30, 0.0, 1.0)
            bad = bad + jnp.where(is_l8, low, 0.0)
        nbad = jnp.sum(bad)

        @pl.when(nbad > 0.0)
        def _():
            def item(t, carry):
                h = lax.shift_right_logical(t, 2)
                q0 = pl.multiple_of(lax.bitwise_and(t, NQ - 1) * BQ, BQ)
                qm = pltpu.bitcast(qh_ref[h, :, pl.ds(q0, BQ)], BF16)

                def chunk(c, st):
                    m, acc = st
                    kl = pltpu.bitcast(
                        kh_ref[h, pl.ds(pl.multiple_of(c * (KC // 2), KC // 2), KC // 2), :], BF16)[:, 0:32]
                    s = lax.dot_general(kl, qm, NN, preferred_element_type=F32)
                    m_new = jnp.maximum(m, jnp.max(s, axis=0, keepdims=True))
                    p = jnp.exp2(s - m_new).astype(BF16)
                    r = lax.dot_general(vt_ref[h, :, pl.ds(pl.multiple_of(c * KC, KC), KC)], p, NN,
                                        preferred_element_type=F32)
                    return m_new, acc * jnp.exp2(m - m_new) + r

                m0 = jnp.full((1, BQ), -jnp.inf, F32)
                _, acc = lax.fori_loop(0, NC, chunk, (m0, jnp.zeros((VROWS, BQ), F32)))
                ot_ref[h, :, pl.ds(q0, BQ)] = acc
                return carry
            lax.fori_loop(0, H * NQ, item, 0)

        for cp in late_copies():
            cp.wait()

    @pl.when(i == 1)
    def _():
        def out_copy(j):
            return pltpu.make_async_copy(ob_ref.at[pl.ds(j * BP, BP), :], o_hbm.at[pl.ds(j * BP, BP), :],
                                         sems.at[SEM_OUT + j])

        row8 = lax.broadcasted_iota(jnp.int32, (8, BP), 0)
        for j in range(NOB):
            rows = slice(j * BP, (j + 1) * BP)
            blocks = []
            for pair in range(H // 2):
                ae = ot_ref[2 * pair, :, rows]
                ao = ot_ref[2 * pair + 1, :, rows]
                rl = _recip(jnp.where(row8 < 4, ao[0:8, :], ae[16:24, :]))
                ae = ae * rl[4:5, :]
                ao = ao * rl[0:1, :]
                blocks.append(ae[0:16, :])
                blocks.append(jnp.where(row8 < 4, ae[16:24, :], ao[0:8, :]))
                blocks.append(ao[8:24, :])
            o = jnp.concatenate(blocks, axis=0).T.astype(BF16)
            a = jnp.dot(o, wo_ref[...], preferred_element_type=F32)
            gw = gw_ref[...].astype(F32).reshape(1, D)
            z = jnp.sum(x_ref[rows, :].astype(F32) * gw, axis=-1, keepdims=True)
            g = 0.5 * jnp.tanh(0.5 * z) + 0.5
            ob_ref[rows, :] = (g * a + (1.0 - g) * b_ref[rows, :]).astype(BF16)
            out_copy(j).start()
        for j in range(NOB):
            out_copy(j).wait()


@jax.jit
def pallas_gated_mix__softmax_full_mha__dense_activation_relu__prompt_kernel(
    A_x: jax.Array,
    A_wqkv: jax.Array,
    A_wo: jax.Array,
    B_x: jax.Array,
    B_w1: jax.Array,
    B_w2: jax.Array,
    gate_w: jax.Array,
):
    del B_x
    anyspec = pl.BlockSpec(memory_space=pl.ANY)
    out = pl.pallas_call(
        _kernel,
        grid=(2,),
        in_specs=[anyspec] * 6,
        out_specs=anyspec,
        out_shape=jax.ShapeDtypeStruct((S, D), BF16),
        scratch_shapes=[
            pltpu.VMEM((S, D), BF16),
            pltpu.VMEM((D, 3 * D), BF16),
            pltpu.VMEM((D, D), BF16),
            pltpu.VMEM((D, DFF), BF16),
            pltpu.VMEM((DFF, D), BF16),
            pltpu.VMEM((D,), BF16),
            pltpu.SemaphoreType.DMA((NSEM,)),
            pltpu.VMEM((H, S // 2, 128), U32),
            pltpu.VMEM((H, VROWS, S), F32),
            pltpu.VMEM((H, 16, S), U32),
            pltpu.VMEM((H, VROWS, S), F32),
            pltpu.VMEM((H, NC // 4 * KG, 128), F32),
            pltpu.VMEM((1, NCT // JB, DH, 8, JB * 128), F32),
            pltpu.VMEM((1, NCT // JB, DH, 8, JB * 128), F32),
            pltpu.VMEM((NSLOT, KC, BQ), F32),
            pltpu.VMEM((H, VROWS, S), F32),
            pltpu.VMEM((2, VROWS + 8, 128), F32),
            pltpu.VMEM((D, D), BF16),
            pltpu.VMEM((128, 512), F32),
            pltpu.VMEM((64, DFF), U32),
            pltpu.VMEM((S, D), F32),
            pltpu.VMEM((S // 2, D), U32),
            pltpu.VMEM((D // 2, DFF), U32),
            pltpu.VMEM((DFF // 2, D), U32),
            pltpu.VMEM((S, D), BF16),
        ] + [pltpu.VMEM((1, 2 if r == 3 else 1, DH, KV, 128), F32) for r in range(NR)],
        compiler_params=pltpu.CompilerParams(
            dimension_semantics=("arbitrary",),
            vmem_limit_bytes=100 * 1024 * 1024),
    )(A_x.reshape(S, D), A_wqkv, A_wo, B_w1, B_w2, gate_w)
    return out.reshape(1, S, D)
```
